```python
import jax
import jax.numpy as jnp

def _softmax(x, axis=-1):
    return jax.nn.softmax(x, axis=axis)

def _gelu(x):
    return jax.nn.gelu(x, approximate=True)

def _silu(x):
    return jax.nn.silu(x)

def _sigmoid(x):
    return jax.nn.sigmoid(x)

def _layernorm(x, axis=-1, eps=1e-05):
    m = jnp.mean(x, axis=axis, keepdims=True)
    v = jnp.var(x, axis=axis, keepdims=True)
    return (x - m) / jnp.sqrt(v + eps)

def _scatter_add(tgt, idx, src, axis=0):
    return tgt.at[idx].add(src)

def _segment_sum(src, seg, n):
    return jax.ops.segment_sum(src, seg, n)

class _Rng:

    def __init__(self, key):
        self._k = key

    def _next(self):
        self._k, sub = jax.random.split(self._k)
        return sub

    def normal(self, shape):
        return jax.random.normal(self._next(), shape, dtype=jnp.bfloat16)

    def randint(self, lo, hi, shape):
        return jax.random.randint(self._next(), shape, lo, hi, dtype=jnp.int32)

    def uniform(self, shape, lo=0.0, hi=1.0):
        return jax.random.uniform(self._next(), shape, jnp.bfloat16, lo, hi)

    def permutation(self, n):
        return jax.random.permutation(self._next(), n)
kernel_name = 'adaLN_cond__sliding_block_cached__mixer_token_mlp__decode'

def setup_inputs():
    _rng = _Rng(jax.random.key(int.from_bytes(__import__("os").urandom(4), "little")))
    _w = lambda a: (lambda t: t.astype(jnp.bfloat16) if jnp.issubdtype(t.dtype, jnp.floating) else t)(jnp.asarray(a))

    def _A_setup():
        B, Sq, D = (1, 1, 640)
        Hq, Hkv, Sk, Dh = (32, 32, 32768, 192)
        assert Hq % Hkv == 0, (Hq, Hkv)
        return {'x': _w((lambda *s: _rng.normal(s) * 0.05)(B, Sq, D)), 'k_cache': _w((lambda *s: _rng.normal(s) * 0.05)(B, Hkv, Sk, Dh)), 'v_cache': _w((lambda *s: _rng.normal(s) * 0.05)(B, Hkv, Sk, Dh)), 'wq': _w((lambda *s: _rng.normal(s) * 0.05)(D, Hq * Dh) * D ** (-0.5)), 'wo': _w((lambda *s: _rng.normal(s) * 0.05)(Hq * Dh, D) * (Hq * Dh) ** (-0.5))}
    _A_in = _A_setup()

    def _B_setup():
        B, S, D, F = (1, 1, 640, 1536)
        return {'x': _w((lambda *s: _rng.normal(s) * 0.05)(B, S, D)), 'w1': _w((lambda *s: _rng.normal(s) * 0.05)(S, F) * S ** (-0.5)), 'b1': _w((lambda *s: _rng.normal(s) * 0.05)(F) * 0.02), 'w2': _w((lambda *s: _rng.normal(s) * 0.05)(F, S) * F ** (-0.5)), 'b2': _w((lambda *s: _rng.normal(s) * 0.05)(S) * 0.02)}
    _B_in = _B_setup()
    return {'A_x': _A_in['x'], 'A_k_cache': _A_in['k_cache'], 'A_v_cache': _A_in['v_cache'], 'A_wq': _A_in['wq'], 'A_wo': _A_in['wo'], 'B_x': _B_in['x'], 'B_w1': _B_in['w1'], 'B_b1': _B_in['b1'], 'B_w2': _B_in['w2'], 'B_b2': _B_in['b2'], 'c': _w((lambda *s: _rng.normal(s) * 0.05)(1, 640)), 'w_mod': _w((lambda *s: _rng.normal(s) * 0.05)(640, 6 * 640) * 640 ** (-0.5))}

def reference(A_x, A_k_cache, A_v_cache, A_wq, A_wo, B_x, B_w1, B_b1, B_w2, B_b2, c, w_mod):

    def _A_ref(x, k_cache, v_cache, wq, wo):
        B, Sq, D = x.shape
        Hq, Dh = (32, 192)
        Hkv, Sk = (k_cache.shape[1], k_cache.shape[2])
        W = min(4096, max(256, Sk // 4))
        rep = Hq // Hkv
        q = (lambda x, *d: x.transpose(*d))((x @ wq).reshape(B, Sq, Hq, Dh), 0, 2, 1, 3)
        k = jnp.repeat(k_cache[:, :, Sk - W:, :], rep, axis=1)
        v = jnp.repeat(v_cache[:, :, Sk - W:, :], rep, axis=1)
        scores = jnp.einsum('bhqd,bhkd->bhqk', q, k) * Dh ** (-0.5)
        p = _softmax(scores, axis=-1)
        o = jnp.einsum('bhqk,bhkd->bhqd', p, v)
        return (lambda x, *d: x.transpose(*d))(o, 0, 2, 1, 3).reshape(B, Sq, Hq * Dh) @ wo

    def _B_ref(x, w1, b1, w2, b2):
        B, S, D = x.shape
        h = _layernorm(x, axis=-1)
        u = jnp.einsum('bsd,sf->bdf', h, w1) + b1
        u = _gelu(u)
        y = jnp.einsum('bdf,fs->bds', u, w2) + b2
        return (lambda x, *d: x.transpose(*d))(y, 0, 2, 1)
    x = A_x
    mod = (_silu(c) @ w_mod).reshape(c.shape[0], 6, 1, -1)
    sa, ca, ga, sb, cb, gb = (mod[:, 0].copy(), mod[:, 1].copy(), mod[:, 2].copy(), mod[:, 3].copy(), mod[:, 4].copy(), mod[:, 5].copy())
    h = _layernorm(x, axis=-1) * (1 + ca) + sa
    x = x + ga * _A_ref(h, A_k_cache, A_v_cache, A_wq, A_wo)
    h = _layernorm(x, axis=-1) * (1 + cb) + sb
    x = x + gb * _B_ref(h, B_w1, B_b1, B_w2, B_b2)
    return x
```

```python
import functools

import jax
import jax.numpy as jnp
from jax import lax
import jax.experimental.pallas as pl
import jax.experimental.pallas.tpu as pltpu

F32 = jnp.float32
BF16 = jnp.bfloat16

D = 640
H = 32
DH = 192
SK = 32768
W = 4096
FF = 1536
EPS = 1e-5

NS = 16
CB = W // NS
HR = 32
NG = DH // 8

WM_C = 5 * D
WM_STEPS = D // 8
WM_HC = 512
WQ_STEPS = D // 8
WQ_HC = 1024
WO_R = 64
WO_STEPS = H * DH // WO_R
WO_HR = 16
GB_R = D // NS
GB_HR = 8


def _layernorm(v):
    m = jnp.mean(v, axis=-1, keepdims=True)
    d = v - m
    var = jnp.mean(d * d, axis=-1, keepdims=True)
    return d * lax.rsqrt(var + EPS)


def _col_bcast(row):
    return jnp.broadcast_to(row, (128, 128)).T


def _tree_sum(xs):
    xs = list(xs)
    while len(xs) > 1:
        nxt = [xs[i] + xs[i + 1] for i in range(0, len(xs) - 1, 2)]
        if len(xs) % 2:
            nxt.append(xs[-1])
        xs = nxt
    return xs[0]


def _kernel(x_hbm, k_hbm, v_hbm, wq_hbm, wo_hbm, w1_hbm, b1_hbm, w2_hbm, b2_hbm, c_hbm, wm_hbm,
            o_ref,
            kbuf, vbuf, wq_v, wo_v, wm_v, x_v, c_v, w1_v, b1_v, w2_v, b2_v,
            qb_ref, s_ref, p_ref, attn_ref, mod_ref, sc_ref, h8_ref, w1c, b1c, w2c,
            sems, ssems):

    def dma(src, dst, slot, prio):
        pltpu.make_async_copy(src, dst, sems.at[slot]).start(priority=prio)

    def wait(dst, slot):
        pltpu.make_async_copy(dst, dst, sems.at[slot]).wait()

    def slot_of(i):
        return i % NS if isinstance(i, int) else lax.rem(i, NS)

    def mult(i, n):
        return i if isinstance(i, int) else pl.multiple_of(i, n)

    def wm_issue(i):
        r = pl.ds(mult(i * 8, 8), 8)
        hi, lo = pl.ds(0, WM_HC), pl.ds(WM_HC, WM_C - WM_HC)
        dma(wm_hbm.at[r, hi], wm_v.at[r, hi], slot_of(i), 0)
        dma(wm_hbm.at[r, lo], wm_v.at[r, lo], slot_of(i), 1)

    def wm_wait(i):
        wait(wm_v.at[pl.ds(mult(i * 8, 8), 8), pl.ds(0, WM_C)], slot_of(i))

    def wq_issue(i):
        r = pl.ds(mult(i * 8, 8), 8)
        hi, lo = pl.ds(0, WQ_HC), pl.ds(WQ_HC, H * DH - WQ_HC)
        dma(wq_hbm.at[r, hi], wq_v.at[r, hi], slot_of(i), 0)
        dma(wq_hbm.at[r, lo], wq_v.at[r, lo], slot_of(i), 1)

    def wq_wait(i):
        wait(wq_v.at[pl.ds(mult(i * 8, 8), 8), :], slot_of(i))

    def wo_issue(i):
        hi = pl.ds(mult(i * WO_R, 8), WO_HR)
        lo = pl.ds(mult(i * WO_R + WO_HR, 8), WO_R - WO_HR)
        dma(wo_hbm.at[hi, :], wo_v.at[hi, :], slot_of(i), 0)
        dma(wo_hbm.at[lo, :], wo_v.at[lo, :], slot_of(i), 1)

    def wo_wait(i):
        wait(wo_v.at[pl.ds(mult(i * WO_R, 8), WO_R), :], slot_of(i))

    def kv_issue(src, buf, h, j):
        c = pl.ds(mult(SK - W + j * CB, 128), CB)
        dma(src.at[pl.ds(mult(h * DH, 8), HR), c], buf.at[j, pl.ds(0, HR), :], j, 0)
        dma(src.at[pl.ds(mult(h * DH + HR, 8), DH - HR), c], buf.at[j, pl.ds(HR, DH - HR), :], j, 1)

    def gb_issue(j):
        c = pl.ds(WM_C, D)
        hi = pl.ds(mult(j * GB_R, 8), GB_HR)
        lo = pl.ds(mult(j * GB_R + GB_HR, 8), GB_R - GB_HR)
        dma(wm_hbm.at[hi, c], wm_v.at[hi, c], j, 0)
        dma(wm_hbm.at[lo, c], wm_v.at[lo, c], j, 1)

    def gb_wait(j):
        wait(wm_v.at[pl.ds(mult(j * GB_R, 8), GB_R), pl.ds(WM_C, D)], j)

    def pump(lo, hi, wait_fn, issue_fn, off):
        def body(i, carry):
            wait_fn(i)
            issue_fn(i + off)
            return carry
        lax.fori_loop(lo, hi, body, 0)

    for i in range(NS):
        wm_issue(i)
    small = [pltpu.make_async_copy(s, d, ssems.at[n]) for n, (s, d) in enumerate(
        [(c_hbm, c_v), (x_hbm, x_v), (w1_hbm, w1_v), (b1_hbm, b1_v), (w2_hbm, w2_v), (b2_hbm, b2_v)])]
    for cp in small:
        cp.start()

    pump(0, WM_STEPS - NS, wm_wait, wm_issue, NS)
    pump(WM_STEPS - NS, WM_STEPS, wm_wait, wq_issue, NS - WM_STEPS)

    for cp in small:
        cp.wait()

    c = c_v[...].astype(F32)
    sc = c * jax.nn.sigmoid(c)
    sc8 = jnp.broadcast_to(sc, (8, D)).astype(BF16)
    sc_ref[...] = sc8
    mod = jnp.dot(sc8, wm_v[:, pl.ds(0, WM_C)], preferred_element_type=F32)
    mod_ref[...] = mod
    x8 = jnp.broadcast_to(x_v[...].astype(F32), (8, D))
    h_in = _layernorm(x8) * (1.0 + mod[:, D:2 * D]) + mod[:, 0:D]
    h8_ref[...] = h_in.astype(BF16)
    attn_ref[...] = jnp.zeros(attn_ref.shape, F32)

    pump(0, NS, wq_wait, wq_issue, NS)
    w1f = w1_v[...].astype(F32)
    for b in range(FF // 128):
        w1c[pl.ds(b * 128, 128), :] = _col_bcast(w1f[:, b * 128:(b + 1) * 128])
    pump(NS, 2 * NS, wq_wait, wq_issue, NS)
    b1f = b1_v[...].astype(F32)
    for b in range(FF // 128):
        b1c[pl.ds(b * 128, 128), :] = _col_bcast(b1f[b:b + 1, :])
    pump(2 * NS, 3 * NS, wq_wait, wq_issue, NS)
    w2f = w2_v[...].astype(F32) * 0.5
    for b in range(FF // 128):
        w2c[pl.ds(b * 128, 128), :] = _col_bcast(w2f[:, b * 128:(b + 1) * 128])
    pump(3 * NS, WQ_STEPS - NS, wq_wait, wq_issue, NS)
    pump(WQ_STEPS - NS, WQ_STEPS, wq_wait, wo_issue, NS - WQ_STEPS)

    QC = H * DH // (WO_STEPS // NS)
    scale = DH ** -0.5

    def q_part(t):
        c0 = mult(t * QC, 128)
        q = jnp.dot(h8_ref[...], wq_v[:, pl.ds(c0, QC)], preferred_element_type=F32)
        q = q.astype(BF16).astype(F32) * scale
        for b in range(QC // 128):
            qb_ref[pl.ds(mult(c0 + b * 128, 128), 128), :] = _col_bcast(q[0:1, b * 128:(b + 1) * 128])

    def wo_round(t, carry):
        q_part(t)
        pump(t * NS, (t + 1) * NS, wo_wait, wo_issue, NS)
        return carry

    lax.fori_loop(0, WO_STEPS // NS - 1, wo_round, 0)
    q_part(WO_STEPS // NS - 1)
    pump(WO_STEPS - NS, WO_STEPS, wo_wait, lambda j: kv_issue(k_hbm, kbuf, 0, j), NS - WO_STEPS)

    def head(h, next_issue):
        r0 = mult(h * DH, 8)

        def kstep(j, carry):
            wait(kbuf.at[j], j)
            kv_issue(v_hbm, vbuf, h, j)
            parts = [[] for _ in range(CB // 128)]
            for g in range(NG):
                kg = kbuf[j, pl.ds(g * 8, 8), :].astype(F32)
                qg = qb_ref[pl.ds(r0 + g * 8, 8), :]
                for cc in range(CB // 128):
                    parts[cc].append(kg[:, cc * 128:(cc + 1) * 128] * qg)
            for cc in range(CB // 128):
                chains = [functools.reduce(lambda a, b: a + b, parts[cc][i::2]) for i in range(2)]
                s_ref[j, :, pl.ds(cc * 128, 128)] = chains[0] + chains[1]
            return carry

        lax.fori_loop(0, NS, kstep, 0)

        s = jnp.sum(s_ref[...], axis=1, keepdims=True)
        m = jnp.max(jnp.max(s, axis=0), axis=1, keepdims=True)
        p = jnp.exp(s - m[None])
        l = jnp.sum(jnp.sum(p, axis=0), axis=1, keepdims=True)
        p_ref[...] = jnp.broadcast_to(p, p_ref.shape)

        def vstep(j, acc):
            wait(vbuf.at[j], j)
            next_issue(j)
            pj = p_ref[j]
            out = []
            for g in range(NG):
                vg = vbuf[j, pl.ds(g * 8, 8), :].astype(F32)
                a = acc[g]
                for cc in range(CB // 128):
                    a = a + vg[:, cc * 128:(cc + 1) * 128] * pj[:, cc * 128:(cc + 1) * 128]
                out.append(a)
            return tuple(out)

        acc = lax.fori_loop(0, NS, vstep, tuple(jnp.zeros((8, 128), F32) for _ in range(NG)))

        inv_l = 1.0 / l
        terms = []
        for g in range(NG):
            og = jnp.sum(acc[g], axis=1, keepdims=True) * inv_l
            terms.append(wo_v[pl.ds(r0 + g * 8, 8), :].astype(F32) * og)
        chains = [functools.reduce(lambda a, b: a + b, terms[i::2]) for i in range(2)]
        attn_ref[...] += chains[0] + chains[1]

    def head_body(h, carry):
        head(h, lambda j: kv_issue(k_hbm, kbuf, h + 1, j))
        return carry

    lax.fori_loop(0, H - 1, head_body, 0)
    head(H - 1, gb_issue)

    attn = jnp.sum(attn_ref[...], axis=0, keepdims=True)
    x = x_v[...].astype(F32)
    x1 = x + mod_ref[0:1, pl.ds(2 * D, D)] * attn
    h2 = _layernorm(x1) * (1.0 + mod_ref[0:1, pl.ds(4 * D, D)]) + mod_ref[0:1, pl.ds(3 * D, D)]
    hn = jnp.broadcast_to(_layernorm(h2), (8, D))
    hs = [hn[:, t * 128:(t + 1) * 128] for t in range(D // 128)]

    k0 = 0.7978845608028654
    k1 = k0 * 0.044715
    FU = 4

    def mlp_body(i, acc):
        acc = list(acc)
        for r in range(FU):
            rows = pl.ds(pl.multiple_of((i * FU + r) * 8, 8), 8)
            a, b, w = w1c[rows, :], b1c[rows, :], w2c[rows, :]
            for t in range(D // 128):
                u = hs[t] * a + b
                th = jnp.tanh(u * (k0 + k1 * (u * u)))
                acc[t] = acc[t] + (u * w) * (1.0 + th)
        return tuple(acc)

    acc = lax.fori_loop(0, FF // (8 * FU), mlp_body, tuple(jnp.zeros((8, 128), F32) for _ in range(D // 128)))
    y = jnp.sum(jnp.concatenate(acc, axis=1), axis=0, keepdims=True) + b2_v[...].astype(F32)

    for j in range(NS):
        gb_wait(j)
    gb = jnp.dot(sc_ref[...], wm_v[:, pl.ds(WM_C, D)], preferred_element_type=F32)
    o_ref[0] = (x1 + gb[0:1, :] * y).astype(o_ref.dtype)


@jax.jit
def pallas_adaLN_cond__sliding_block_cached__mixer_token_mlp__decode_kernel(
    A_x: jax.Array,
    A_k_cache: jax.Array,
    A_v_cache: jax.Array,
    A_wq: jax.Array,
    A_wo: jax.Array,
    B_x: jax.Array,
    B_w1: jax.Array,
    B_b1: jax.Array,
    B_w2: jax.Array,
    B_b2: jax.Array,
    c: jax.Array,
    w_mod: jax.Array,
):
    del B_x
    kt = jnp.swapaxes(A_k_cache, 2, 3).reshape(H * DH, SK)
    vt = jnp.swapaxes(A_v_cache, 2, 3).reshape(H * DH, SK)
    args = (A_x.reshape(1, D), kt, vt, A_wq, A_wo, B_w1, B_b1.reshape(FF // 128, 128),
            B_w2.reshape(1, FF), B_b2, c, w_mod)
    scratch = [
        pltpu.VMEM((NS, DH, CB), BF16),
        pltpu.VMEM((NS, DH, CB), BF16),
        pltpu.VMEM((D, H * DH), BF16),
        pltpu.VMEM((H * DH, D), BF16),
        pltpu.VMEM((D, 6 * D), BF16),
        pltpu.VMEM((1, D), BF16),
        pltpu.VMEM((1, D), BF16),
        pltpu.VMEM((1, FF), BF16),
        pltpu.VMEM((FF // 128, 128), BF16),
        pltpu.VMEM((1, FF), BF16),
        pltpu.VMEM((1,), BF16),
        pltpu.VMEM((H * DH, 128), F32),
        pltpu.VMEM((NS, 8, CB), F32),
        pltpu.VMEM((NS, 8, CB), F32),
        pltpu.VMEM((8, D), F32),
        pltpu.VMEM((8, WM_C), F32),
        pltpu.VMEM((8, D), BF16),
        pltpu.VMEM((8, D), BF16),
        pltpu.VMEM((FF, 128), F32),
        pltpu.VMEM((FF, 128), F32),
        pltpu.VMEM((FF, 128), F32),
        pltpu.SemaphoreType.DMA((NS,)),
        pltpu.SemaphoreType.DMA((6,)),
    ]
    return pl.pallas_call(
        _kernel,
        in_specs=[pl.BlockSpec(memory_space=pl.ANY)] * len(args),
        out_specs=pl.BlockSpec(memory_space=pltpu.VMEM),
        out_shape=jax.ShapeDtypeStruct((1, 1, D), BF16),
        scratch_shapes=scratch,
        compiler_params=pltpu.CompilerParams(
            vmem_limit_bytes=120 * 1024 * 1024,
            disable_bounds_checks=True,
            disable_semaphore_checks=True,
        ),
    )(*args)
```

```python
import functools

import jax
import jax.numpy as jnp
from jax import lax
import jax.experimental.pallas as pl
import jax.experimental.pallas.tpu as pltpu

F32 = jnp.float32
BF16 = jnp.bfloat16

D = 640
H = 32
DH = 192
SK = 32768
W = 4096
FF = 1536
EPS = 1e-5
NT = D // 128
NC = FF // 128

NS = 16
CB = W // NS
HR = 32
NG = DH // 8

GM = 10
RM = D // GM
GO = 8
RO = H * DH // GO
GH = 2
WM_G = 5
WM_STEPS = WM_G * (RM // 8)
WQ_C = 384
WQ_STEPS = (H * DH // WQ_C) * (RM // 8)
WO_STEPS = RO // 8
LR = 16
LN_STEPS = DH // LR
LHC = 512
MLPSPLIT = 10
NV = 128
GBH = 0
KS = 8
GBPOS = 2
NVC = 2
NV1 = 0
SEG = 4
NOTAIL = 0
SKIPKV = 0
NOTASK = 0
GBEARLY = 0
TAILONLY = 0

GELU_K0 = 0.7978845608028654
GELU_K1 = GELU_K0 * 0.044715
GELU_S = GELU_K1 ** (1.0 / 3.0)
GELU_KAPPA = GELU_K0 / GELU_S

V_X, V_XN, V_SA, V_CA, V_GA, V_SB, V_CB, V_Y, V_MISC = range(9)


def _lane_mean(v):
    return jnp.sum(v, axis=-1, keepdims=True) * (1.0 / D)


def _col_bcast(row):
    return jnp.broadcast_to(row, (128, 128)).T


def _chain_sum(xs, n):
    chains = [functools.reduce(lambda a, b: a + b, xs[i::n]) for i in range(n)]
    while len(chains) > 1:
        chains = [chains[i] + chains[i + 1] for i in range(0, len(chains), 2)]
    return chains[0]


def _sub_allreduce(v):
    v = v + pltpu.roll(v, 4, 0)
    v = v + pltpu.roll(v, 2, 0)
    return v + pltpu.roll(v, 1, 0)


def _tile(v, t):
    return v[:, t * 128:(t + 1) * 128]


def _kernel(x_hbm, k_hbm, v_hbm, wq_hbm, wo_hbm, w1_hbm, b1_hbm, w2_hbm, b2_hbm, c_hbm, wm_hbm,
            o_ref,
            kbuf, vbuf, vlast, wq_v, wo_v, wm_v, x_v, c_v, w1_v, b1_v, w2_v, b2_v,
            qb_ref, s_ref, p_ref, attn_ref, vec_ref, sc_ref, h8_ref, w1c, b1c, w2c, th_ref, ab_ref, wol_ref,
            sems, ssems, gsem):

    def dma(src, dst, sem, prio):
        pltpu.make_async_copy(src, dst, sem).start(priority=prio)

    def wait(dst, sem):
        pltpu.make_async_copy(dst, dst, sem).wait()

    def static(i):
        return isinstance(i, int)

    def mult(i, n):
        return i if static(i) else pl.multiple_of(i, n)

    def rem(i, n):
        return i % n if static(i) else lax.rem(i, n)

    def div(i, n):
        return i // n if static(i) else lax.div(i, n)

    def weight_steps(hbm, vmem, groups, ncols, ncb, base):
        def where(i):
            if ncb == 1:
                return pl.ds(mult(i * 8, 8), 8), pl.ds(0, ncols)
            return pl.ds(mult(div(i, ncb) * 8, 8), 8), pl.ds(mult(rem(i, ncb) * ncols, 128), ncols)

        def issue(i):
            r, c = where(i)
            sem = sems.at[rem(i + base, NS)]
            hi, lo = pl.ds(0, GH), pl.ds(GH, groups - GH)
            dma(hbm.at[hi, r, c], vmem.at[hi, r, c], sem, 0)
            dma(hbm.at[lo, r, c], vmem.at[lo, r, c], sem, 1)

        def wait_(i):
            r, c = where(i)
            wait(vmem.at[:, r, c], sems.at[rem(i + base, NS)])

        return issue, wait_

    base_wm = (-(WM_STEPS + WQ_STEPS + WO_STEPS)) % NS
    wm_issue, wm_wait = weight_steps(wm_hbm, wm_v, GM, D, WM_G, base_wm)
    wq_issue, wq_wait = weight_steps(wq_hbm, wq_v, GM, WQ_C, H * DH // WQ_C, (base_wm + WM_STEPS) % NS)
    wo_issue, wo_wait = weight_steps(wo_hbm, wo_v, GO, D, 1, (base_wm + WM_STEPS + WQ_STEPS) % NS)

    def kv_issue(src, buf, h, j):
        c = pl.ds(mult(SK - W + j * CB, 128), CB)
        dma(src.at[pl.ds(mult(h * DH, 8), HR), c], buf.at[j, pl.ds(0, HR), :], sems.at[j], 0)
        dma(src.at[pl.ds(mult(h * DH + HR, 8), DH - HR), c], buf.at[j, pl.ds(HR, DH - HR), :], sems.at[j], 1)

    def vlast_issue(j):
        rs = pl.ds(mult((H - 1) * DH + j * LR, 8), LR)
        rd = pl.ds(mult(j * LR, 8), LR)
        dma(v_hbm.at[rs, pl.ds(SK - W, LHC)], vlast.at[rd, pl.ds(0, LHC)], sems.at[j], 0)
        dma(v_hbm.at[rs, pl.ds(SK - W + LHC, W - LHC)], vlast.at[rd, pl.ds(LHC, W - LHC)], sems.at[j], 1)

    def gb_issue(j):
        r, c = pl.ds(mult(j * 8, 8), 8), pl.ds(WM_G * D, D)
        hi, lo = pl.ds(0, GBH), pl.ds(GBH, GM - GBH)
        if GBH:
            dma(wm_hbm.at[hi, r, c], wm_v.at[hi, r, c], gsem, 0)
        dma(wm_hbm.at[lo, r, c], wm_v.at[lo, r, c], gsem, 1)

    def pump(lo, hi, wait_fn, issue_fn, off):
        def body(i, carry):
            wait_fn(i)
            issue_fn(i + off)
            return carry
        if hi > lo:
            lax.fori_loop(lo, hi, body, 0)

    def phase(n, wait_fn, issue_fn, next_issue, tasks):
        i = 0
        for task in tasks:
            pump(i, i + SEG, wait_fn, issue_fn, NS)
            i += SEG
            assert i <= n - NS
            if not NOTASK:
                task()
        pump(i, n - NS, wait_fn, issue_fn, NS)
        pump(n - NS, n, wait_fn, next_issue, NS - n)

    def main_part():
        for i in range(NS):
            wm_issue(i)
        small = [pltpu.make_async_copy(s, d, ssems.at[n]) for n, (s, d) in enumerate(
            [(c_hbm, c_v), (x_hbm, x_v), (w1_hbm, w1_v), (b1_hbm, b1_v), (w2_hbm, w2_v), (b2_hbm, b2_v)])]
        for cp in small:
            cp.start()

        def first_task():
            c = c_v[...].astype(F32)
            sc_ref[...] = jnp.broadcast_to(c * jax.nn.sigmoid(c), (8, D)).astype(BF16)
            x8 = jnp.broadcast_to(x_v[...].astype(F32), (8, D))
            xc = x8 - _lane_mean(x8)
            vec_ref[V_X] = x8
            vec_ref[V_XN] = xc * lax.rsqrt(_lane_mean(xc * xc) + EPS)
            attn_ref[...] = jnp.zeros(attn_ref.shape, F32)
            w2f = w2_v[...].astype(F32) * 0.5
            w1r = w1_v[...].astype(F32)
            b1r = b1_v[...].astype(F32)
            row = lax.broadcasted_iota(jnp.int32, (8, 128), 0)
            sum_ab = jnp.zeros((8, 128), F32)
            for b in range(NC):
                wa = _tile(w2f, b) * _tile(w1r, b)
                wb = _tile(w2f, b) * b1r[b:b + 1, :]
                ab = jnp.where(row < 2, jnp.broadcast_to(wa, (8, 128)), jnp.broadcast_to(wb, (8, 128)))
                ab = jnp.where(row < 4, ab, 0.0)
                hi = ab.astype(BF16).astype(F32)
                ab_ref[:, pl.ds(b * 128, 128)] = jnp.where(row % 2 == 0, hi, (ab - hi).astype(BF16).astype(F32))
                sum_ab = sum_ab + jnp.where(row % 2 == 0, ab, 0.0)
            sum_ab = jnp.broadcast_to(jnp.sum(sum_ab, axis=1, keepdims=True), (8, 128))
            b2 = jnp.broadcast_to(b2_v[...].astype(F32), (8, 128))
            vec_ref[V_MISC, :, pl.ds(0, 128)] = sum_ab + jnp.where(row == 2, b2, 0.0)

        def col_task(b0, nb):
            def task():
                w1f = w1_v[...].astype(F32) * GELU_S
                b1f = b1_v[...].astype(F32) * GELU_S
                for b in range(b0, b0 + nb):
                    w1c[pl.ds(b * 128, 128), :] = _col_bcast(_tile(w1f, b))
                    b1c[pl.ds(b * 128, 128), :] = _col_bcast(b1f[b:b + 1, :])
                if b0 // 2 < NVC + 1:
                    w2c[pl.ds((b0 // 2) * 128, 128), :] = _col_bcast(_tile(w2_v[...].astype(F32) * (0.5 / GELU_S), NC - NVC - 1 + b0 // 2))
            return task

        def mod_task(n):
            def task():
                w = wm_v[:, :, pl.ds(n * D, D)].reshape(D, D)
                vec_ref[V_SA + n] = jnp.dot(sc_ref[...], w, preferred_element_type=F32)
            return task

        def h_task():
            h8_ref[...] = (vec_ref[V_XN] * (1.0 + vec_ref[V_CA]) + vec_ref[V_SA]).astype(BF16)
            sb = vec_ref[V_SB]
            st = sb - _lane_mean(sb)
            vec_ref[V_SB] = st
            vec_ref[V_CB] = 1.0 + vec_ref[V_CB]
            vec_ref[V_MISC, :, pl.ds(128, 128)] = jnp.broadcast_to(_lane_mean(st * st) + EPS, (8, 128))

        def q_cols(h):
            c0 = mult(div(h * DH, 128) * 128, 128)
            q = jnp.dot(h8_ref[...], wq_v[:, :, pl.ds(c0, 256)].reshape(D, 256), preferred_element_type=F32)
            q = q.astype(BF16).astype(F32) * (DH ** -0.5)
            for b in range(2):
                qb_ref[pl.ds(b * 128, 128), :] = _col_bcast(_tile(q, b)[0:1])

        def small_wait():
            for cp in small:
                cp.wait()

        pump(0, SEG, wm_wait, wm_issue, NS)
        small_wait()
        first_task()
        pump(SEG, WM_STEPS - NS, wm_wait, wm_issue, NS)
        pump(WM_STEPS - NS, WM_STEPS, wm_wait, wq_issue, NS - WM_STEPS)
        phase(WQ_STEPS, wq_wait, wq_issue, wo_issue,
              [mod_task(n) for n in range(WM_G)] + [h_task] + [col_task(b, 2) for b in range(0, NC, 2)])
        phase(WO_STEPS, wo_wait, wo_issue, lambda j: kv_issue(k_hbm, kbuf, 0, j), [lambda: q_cols(0)])

        for g in range(NG):
            wg = wo_v[GO - 1, pl.ds(RO - DH + g * 8, 8), :].astype(F32) * vec_ref[V_GA]
            mg = _lane_mean(wg)
            wol_ref[pl.ds(g * 8, 8), pl.ds(0, D)] = wg - mg
            wol_ref[pl.ds(g * 8, 8), pl.ds(D, 128)] = jnp.broadcast_to(mg, (8, 128))

        if GBEARLY:
            for j in range(RM // 8):
                gb_issue(j)
        def scores(h, issue):
            r0 = mult(rem(h * DH, 128), 64)

            def kstep(j, carry):
                wait(kbuf.at[j], sems.at[j])
                issue(j)
                parts = [[] for _ in range(CB // 128)]
                for g in range(NG):
                    kg = kbuf[j, pl.ds(g * 8, 8), :].astype(F32)
                    qg = qb_ref[pl.ds(r0 + g * 8, 8), :]
                    for cc in range(CB // 128):
                        parts[cc].append(_tile(kg, cc) * qg)
                for cc in range(CB // 128):
                    s_ref[j, :, pl.ds(cc * 128, 128)] = _chain_sum(parts[cc], 2)
                return carry

            lax.fori_loop(0, NS, kstep, 0)

            s = jnp.sum(s_ref[...], axis=1, keepdims=True)
            m = jnp.max(jnp.max(s, axis=0), axis=1, keepdims=True)
            p = jnp.exp(s - m[None])
            l = jnp.sum(jnp.sum(p, axis=0), axis=1, keepdims=True)
            p_ref[...] = jnp.broadcast_to(p, p_ref.shape)
            return 1.0 / l

        def head_body(h, carry):
            inv_l = scores(h, lambda j: kv_issue(v_hbm, vbuf, h, j))
            q_cols(h + 1)

            def vstep(j, acc):
                wait(vbuf.at[j], sems.at[j])
                kv_issue(k_hbm, kbuf, h + 1, j)
                pj = p_ref[j]
                out = []
                for g in range(NG):
                    vg = vbuf[j, pl.ds(g * 8, 8), :].astype(F32)
                    a = acc[g]
                    for cc in range(CB // 128):
                        a = a + _tile(vg, cc) * _tile(pj, cc)
                    out.append(a)
                return tuple(out)

            acc = lax.fori_loop(0, NS, vstep, tuple(jnp.zeros((8, 128), F32) for _ in range(NG)))

            hg = div(h, H // GO)
            r0 = mult(rem(h, H // GO) * DH, 8)
            terms = []
            for g in range(NG):
                og = jnp.sum(acc[g], axis=1, keepdims=True) * inv_l
                terms.append(wo_v[hg, pl.ds(r0 + g * 8, 8), :].astype(F32) * og)
            attn_ref[...] += _chain_sum(terms, 2)
            return carry

        lax.fori_loop(0, H - 1 - SKIPKV, head_body, 0)

        def last_issue(j):
            @pl.when(j < LN_STEPS)
            def _():
                vlast_issue(j)

        inv_l = scores(H - 1, last_issue)

        xp = vec_ref[V_X] + vec_ref[V_GA] * _sub_allreduce(attn_ref[...])
        mp = _lane_mean(xp)
        vec_ref[V_Y] = xp - mp
        vec_ref[V_MISC, :, pl.ds(256, 128)] = jnp.broadcast_to(mp, (8, 128))

        def lstep(j, acc):
            rows = mult(j * LR, 8)
            wait(vlast.at[pl.ds(rows, LR), :], sems.at[j])

            if not GBEARLY:
                @pl.when(j < RM // 8)
                def _():
                    gb_issue(j)

            for g in range(LR // 8):
                parts = []
                for t in range(NS):
                    vg = vlast[pl.ds(rows + g * 8, 8), pl.ds(t * CB, CB)].astype(F32)
                    pv = vg * p_ref[t]
                    parts += [_tile(pv, cc) for cc in range(CB // 128)]
                og = jnp.sum(_chain_sum(parts, 4), axis=1, keepdims=True) * inv_l
                acc = acc + wol_ref[pl.ds(rows + g * 8, 8), :] * og
            return acc

        acc = lax.fori_loop(0, LN_STEPS, lstep, jnp.zeros((8, D + 128), F32))

        return acc

    if TAILONLY:
        for j in range(RM // 8):
            gb_issue(j)
        pl.delay(2000)
        acc = wol_ref[pl.ds(0, 8), :]
    else:
        acc = main_part()

    if NOTAIL:
        wait(wm_v.at[:, :, pl.ds(WM_G * D, D)], gsem)
        o_ref[0] = acc[0:1, 0:D].astype(o_ref.dtype)
        return

    acc = _sub_allreduce(acc)
    y = vec_ref[V_Y] + acc[:, 0:D]
    m1 = vec_ref[V_MISC, :, pl.ds(256, 128)] + acc[:, D:D + 128]
    st = vec_ref[V_SB]
    yg = y * vec_ref[V_CB]
    r1 = lax.rsqrt(_lane_mean(y * y) + EPS)
    m2 = _lane_mean(yg)
    v2 = _lane_mean(yg * yg) - m2 * m2
    cv = _lane_mean(yg * st)
    r2 = lax.rsqrt(r1 * (r1 * v2 + 2.0 * cv) + vec_ref[V_MISC, :, pl.ds(128, 128)])
    r12 = r1 * r2
    hs = [(_tile(yg, t) - m2) * r12 + _tile(st, t) * r2 for t in range(NT)]

    def hidden(t, r0, n):
        a = w1c[pl.ds(r0, n), :].reshape(n // 8, 8, 128)
        b = b1c[pl.ds(r0, n), :].reshape(n // 8, 8, 128)
        v = hs[t][None] * a + b
        return v, jnp.tanh(v * (v * v + GELU_KAPPA))

    def contract(t, r0, n, th):
        return jnp.dot(ab_ref[:, pl.ds(r0, n)], th, preferred_element_type=F32, precision=lax.Precision.DEFAULT)

    W2_0 = (NC - NVC - 1) * 128

    def vpu_rows(r0, n, accv):
        for r in range(r0, r0 + n, 8):
            a, b, w = w1c[pl.ds(r, 8), :], b1c[pl.ds(r, 8), :], w2c[pl.ds(r - W2_0, 8), :]
            for t in range(NT):
                v = hs[t] * a + b
                g = (v * jnp.tanh(v * (v * v + GELU_KAPPA))) * w
                accv[t] = g if accv[t] is None else accv[t] + g
        return accv

    R2 = FF - NV - NV1
    R1 = min(MLPSPLIT * 128, R2)
    units = [(t, r0, min(128, R2 - r0)) for r0 in range(0, R2, 128) for t in range(NT)]
    n1 = len([u for u in units if u[1] < R1])
    acc = [vec_ref[V_MISC, :, pl.ds(0, 128)]] * NT
    accv = [None] * NT
    for k, (t, r0, n) in enumerate(units[:n1]):
        th = hidden(t, r0, n)[1].reshape(n, 128)
        if k < n1 - KS:
            acc[t] = acc[t] + contract(t, r0, n, th)
        else:
            th_ref[k - (n1 - KS), pl.ds(0, n), :] = th
    accv = vpu_rows(R2, NV1, accv)
    wait(wm_v.at[:, :, pl.ds(WM_G * D, D)], gsem)

    def gb_tile(t):
        return jnp.dot(sc_ref[...], wm_v[:, :, pl.ds(WM_G * D + t * 128, 128)].reshape(D, 128), preferred_element_type=F32)

    gb = []
    if GBPOS == 0:
        gb = [gb_tile(t) for t in range(NT)]
    for k, (t, r0, n) in enumerate(units[n1 - KS:n1]):
        acc[t] = acc[t] + contract(t, r0, n, th_ref[k, pl.ds(0, n), :])
    if GBPOS == 1:
        gb = [gb_tile(t) for t in range(NT)]
    for k, (t, r0, n) in enumerate(units[n1:]):
        acc[t] = acc[t] + contract(t, r0, n, hidden(t, r0, n)[1].reshape(n, 128))
        if GBPOS == 2 and len(gb) < NT:
            gb.append(gb_tile(len(gb)))
    while len(gb) < NT:
        gb.append(gb_tile(len(gb)))
    accv = vpu_rows(R2 + NV1, NV, accv)
    row = lax.broadcasted_iota(jnp.int32, (8, 128), 0)
    outs = []
    for t in range(NT):
        yt = acc[t] * jnp.where(row < 2, hs[t], 1.0)
        if accv[t] is not None:
            yt = yt + accv[t]
        outs.append(_tile(y, t) + m1 + gb[t] * _sub_allreduce(yt))
    o_ref[0] = jnp.concatenate(outs, axis=1)[0:1, :].astype(o_ref.dtype)


@jax.jit
def pallas_adaLN_cond__sliding_block_cached__mixer_token_mlp__decode_kernel(
    A_x: jax.Array,
    A_k_cache: jax.Array,
    A_v_cache: jax.Array,
    A_wq: jax.Array,
    A_wo: jax.Array,
    B_x: jax.Array,
    B_w1: jax.Array,
    B_b1: jax.Array,
    B_w2: jax.Array,
    B_b2: jax.Array,
    c: jax.Array,
    w_mod: jax.Array,
):
    del B_x
    kt = jnp.swapaxes(A_k_cache, 2, 3).reshape(H * DH, SK)
    vt = jnp.swapaxes(A_v_cache, 2, 3).reshape(H * DH, SK)
    args = (A_x.reshape(1, D), kt, vt, A_wq.reshape(GM, RM, H * DH), A_wo.reshape(GO, RO, D), B_w1,
            B_b1.reshape(NC, 128), B_w2.reshape(1, FF), B_b2, c, w_mod.reshape(GM, RM, 6 * D))
    scratch = [
        pltpu.VMEM((NS, DH, CB), BF16),
        pltpu.VMEM((NS, DH, CB), BF16),
        pltpu.VMEM((DH, W), BF16),
        pltpu.VMEM((GM, RM, H * DH), BF16),
        pltpu.VMEM((GO, RO, D), BF16),
        pltpu.VMEM((GM, RM, 6 * D), BF16),
        pltpu.VMEM((1, D), BF16),
        pltpu.VMEM((1, D), BF16),
        pltpu.VMEM((1, FF), BF16),
        pltpu.VMEM((NC, 128), BF16),
        pltpu.VMEM((1, FF), BF16),
        pltpu.VMEM((1,), BF16),
        pltpu.VMEM((256, 128), F32),
        pltpu.VMEM((NS, 8, CB), F32),
        pltpu.VMEM((NS, 8, CB), F32),
        pltpu.VMEM((8, D), F32),
        pltpu.VMEM((9, 8, D), F32),
        pltpu.VMEM((8, D), BF16),
        pltpu.VMEM((8, D), BF16),
        pltpu.VMEM((FF, 128), F32),
        pltpu.VMEM((FF, 128), F32),
        pltpu.VMEM(((NVC + 1) * 128, 128), F32),
        pltpu.VMEM((max(KS, 1), 128, 128), F32),
        pltpu.VMEM((8, FF), F32),
        pltpu.VMEM((DH, D + 128), F32),
        pltpu.SemaphoreType.DMA((NS,)),
        pltpu.SemaphoreType.DMA((6,)),
        pltpu.SemaphoreType.DMA(()),
    ]
    return pl.pallas_call(
        _kernel,
        in_specs=[pl.BlockSpec(memory_space=pl.ANY)] * len(args),
        out_specs=pl.BlockSpec(memory_space=pltpu.VMEM),
        out_shape=jax.ShapeDtypeStruct((1, 1, D), BF16),
        scratch_shapes=scratch,
        compiler_params=pltpu.CompilerParams(
            vmem_limit_bytes=120 * 1024 * 1024,
            disable_bounds_checks=True,
            disable_semaphore_checks=True,
        ),
    )(*args)
```

```python
import functools

import jax
import jax.numpy as jnp
from jax import lax
import jax.experimental.pallas as pl
import jax.experimental.pallas.tpu as pltpu

F32 = jnp.float32
BF16 = jnp.bfloat16

D = 640
H = 32
DH = 192
SK = 32768
W = 4096
FF = 1536
EPS = 1e-5
NT = D // 128
NC = FF // 128
NG = DH // 8

CB = 128
NB = W // CB
HR = 16

NS = 16
GM = 10
RM = D // GM
GO = 8
RO = H * DH // GO
GH = 2
WM_G = 5
WM_STEPS = WM_G * (RM // 8)
WQ_C = 384
WQ_STEPS = (H * DH // WQ_C) * (RM // 8)
WO_STEPS = RO // 8
SEG = 4

LR = 16
LN_STEPS = DH // LR
LHC = 256

MLP_SPLIT = 10
KS = 5
NV = 96

GELU_K0 = 0.7978845608028654
GELU_K1 = GELU_K0 * 0.044715
GELU_S = GELU_K1 ** (1.0 / 3.0)
GELU_KAPPA = GELU_K0 / GELU_S

V_X, V_XN, V_SA, V_CA, V_GA, V_SB, V_CB, V_Y, V_MISC = range(9)


def _lane_mean(v):
    return jnp.sum(v, axis=-1, keepdims=True) * (1.0 / D)


def _col_bcast(row):
    return jnp.broadcast_to(row, (128, 128)).T


def _chain_sum(xs, n):
    chains = [functools.reduce(lambda a, b: a + b, xs[i::n]) for i in range(n)]
    while len(chains) > 1:
        chains = [chains[i] + chains[i + 1] for i in range(0, len(chains), 2)]
    return chains[0]


def _sub_allreduce(v):
    v = v + pltpu.roll(v, 4, 0)
    v = v + pltpu.roll(v, 2, 0)
    return v + pltpu.roll(v, 1, 0)


def _tile(v, t):
    return v[:, t * 128:(t + 1) * 128]


def _mult(i, n):
    return i if isinstance(i, int) else pl.multiple_of(i, n)


def _rem(i, n):
    return i % n if isinstance(i, int) else lax.rem(i, n)


def _div(i, n):
    return i // n if isinstance(i, int) else lax.div(i, n)


def _kernel(x_hbm, k_hbm, v_hbm, wq_hbm, wo_hbm, w1_hbm, b1_hbm, w2_hbm, b2_hbm, c_hbm, wm_hbm,
            o_ref,
            kbuf, vbuf, vlast, wq_v, wo_v, wm_v, gb_v, x_v, c_v, w1_v, b1_v, w2_v, b2_v,
            qb_ref, s_ref, p_ref, attn_ref, vec_ref, sc_ref, h8_ref, w1c, b1c, w2c, ab_ref, wol_ref,
            sems, kvs, ssems, gsem):

    def dma(src, dst, sem, prio):
        pltpu.make_async_copy(src, dst, sem).start(priority=prio)

    def wait(dst, sem):
        pltpu.make_async_copy(dst, dst, sem).wait()

    def weight_steps(hbm, vmem, groups, ncols, ncb, base):
        def where(i):
            if ncb == 1:
                return pl.ds(_mult(i * 8, 8), 8), pl.ds(0, ncols)
            return pl.ds(_mult(_div(i, ncb) * 8, 8), 8), pl.ds(_mult(_rem(i, ncb) * ncols, 128), ncols)

        def issue(i):
            r, c = where(i)
            sem = sems.at[_rem(i + base, NS)]
            hi, lo = pl.ds(0, GH), pl.ds(GH, groups - GH)
            dma(hbm.at[hi, r, c], vmem.at[hi, r, c], sem, 0)
            dma(hbm.at[lo, r, c], vmem.at[lo, r, c], sem, 1)

        def wait_(i):
            r, c = where(i)
            wait(vmem.at[:, r, c], sems.at[_rem(i + base, NS)])

        return issue, wait_

    wm_issue, wm_wait = weight_steps(wm_hbm, wm_v, GM, D, WM_G, 0)
    wq_issue, wq_wait = weight_steps(wq_hbm, wq_v, GM, WQ_C, H * DH // WQ_C, WM_STEPS % NS)
    wo_issue, wo_wait = weight_steps(wo_hbm, wo_v, GO, D, 1, (WM_STEPS + WQ_STEPS) % NS)

    def kv_issue(src, buf, h, j):
        c = pl.ds(_mult(SK - W + j * CB, 128), CB)
        dma(src.at[pl.ds(_mult(h * DH, 8), HR), c], buf.at[j, pl.ds(0, HR), :], kvs.at[j], 0)
        dma(src.at[pl.ds(_mult(h * DH + HR, 8), DH - HR), c], buf.at[j, pl.ds(HR, DH - HR), :], kvs.at[j], 1)

    def k0_issue(j):
        for u in range(NB // NS):
            kv_issue(k_hbm, kbuf, 0, j * (NB // NS) + u)

    def vlast_issue(j):
        rs = pl.ds(_mult((H - 1) * DH + j * LR, 8), LR)
        rd = pl.ds(_mult(j * LR, 8), LR)
        dma(v_hbm.at[rs, pl.ds(SK - W, LHC)], vlast.at[rd, pl.ds(0, LHC)], sems.at[j], 0)
        dma(v_hbm.at[rs, pl.ds(SK - W + LHC, W - LHC)], vlast.at[rd, pl.ds(LHC, W - LHC)], sems.at[j], 1)

    def gb_issue(j):
        r = pl.ds(_mult(j * 8, 8), 8)
        dma(wm_hbm.at[:, r, pl.ds(WM_G * D, D)], gb_v.at[:, r, :], gsem, 1)

    def pump(lo, hi, wait_fn, issue_fn, off):
        def body(i, carry):
            wait_fn(i)
            issue_fn(i + off)
            return carry
        lax.fori_loop(lo, hi, body, 0)

    def phase(n, wait_fn, issue_fn, next_issue, tasks):
        for k, task in enumerate(tasks):
            pump(k * SEG, (k + 1) * SEG, wait_fn, issue_fn, NS)
            task()
        pump(len(tasks) * SEG, n - NS, wait_fn, issue_fn, NS)
        pump(n - NS, n, wait_fn, next_issue, NS - n)

    for i in range(NS):
        wm_issue(i)
    small = [pltpu.make_async_copy(s, d, ssems.at[n]) for n, (s, d) in enumerate(
        [(c_hbm, c_v), (x_hbm, x_v), (w1_hbm, w1_v), (b1_hbm, b1_v), (w2_hbm, w2_v), (b2_hbm, b2_v)])]
    for cp in small:
        cp.start()

    def first_task():
        for cp in small:
            cp.wait()
        c = c_v[...].astype(F32)
        sc_ref[...] = jnp.broadcast_to(c * jax.nn.sigmoid(c), (8, D)).astype(BF16)
        x8 = jnp.broadcast_to(x_v[...].astype(F32), (8, D))
        xc = x8 - _lane_mean(x8)
        vec_ref[V_X] = x8
        vec_ref[V_XN] = xc * lax.rsqrt(_lane_mean(xc * xc) + EPS)
        attn_ref[...] = jnp.zeros(attn_ref.shape, F32)
        w2f = w2_v[...].astype(F32) * 0.5
        w1r = w1_v[...].astype(F32)
        b1r = b1_v[...].astype(F32)
        row = lax.broadcasted_iota(jnp.int32, (8, 128), 0)
        sum_ab = jnp.zeros((8, 128), F32)
        for b in range(NC):
            wa = _tile(w2f, b) * _tile(w1r, b)
            wb = _tile(w2f, b) * b1r[b:b + 1, :]
            ab = jnp.where(row < 2, jnp.broadcast_to(wa, (8, 128)), jnp.broadcast_to(wb, (8, 128)))
            ab = jnp.where(row < 4, ab, 0.0)
            hi = ab.astype(BF16).astype(F32)
            ab_ref[:, pl.ds(b * 128, 128)] = jnp.where(row % 2 == 0, hi, (ab - hi).astype(BF16).astype(F32))
            sum_ab = sum_ab + jnp.where(row % 2 == 0, ab, 0.0)
        sum_ab = jnp.broadcast_to(jnp.sum(sum_ab, axis=1, keepdims=True), (8, 128))
        b2 = jnp.broadcast_to(b2_v[...].astype(F32), (8, 128))
        vec_ref[V_MISC, :, pl.ds(0, 128)] = sum_ab + jnp.where(row == 2, b2, 0.0)

    def col_task(b0, nb):
        def task():
            w1f = w1_v[...].astype(F32) * GELU_S
            b1f = b1_v[...].astype(F32) * GELU_S
            for b in range(b0, b0 + nb):
                w1c[pl.ds(b * 128, 128), :] = _col_bcast(_tile(w1f, b))
                b1c[pl.ds(b * 128, 128), :] = _col_bcast(b1f[b:b + 1, :])
            if b0 == 0:
                w2c[...] = _col_bcast(_tile(w2_v[...].astype(F32) * (0.5 / GELU_S), NC - 1))
        return task

    def mod_task(n):
        def task():
            w = wm_v[:, :, pl.ds(n * D, D)].reshape(D, D)
            vec_ref[V_SA + n] = jnp.dot(sc_ref[...], w, preferred_element_type=F32)
        return task

    def h_task():
        h8_ref[...] = (vec_ref[V_XN] * (1.0 + vec_ref[V_CA]) + vec_ref[V_SA]).astype(BF16)
        sb = vec_ref[V_SB]
        st = sb - _lane_mean(sb)
        vec_ref[V_SB] = st
        vec_ref[V_CB] = 1.0 + vec_ref[V_CB]
        vec_ref[V_MISC, :, pl.ds(128, 128)] = jnp.broadcast_to(_lane_mean(st * st) + EPS, (8, 128))

    def q_cols(h):
        c0 = _mult(_div(h * DH, 128) * 128, 128)
        q = jnp.dot(h8_ref[...], wq_v[:, :, pl.ds(c0, 256)].reshape(D, 256), preferred_element_type=F32)
        q = q.astype(BF16).astype(F32) * (DH ** -0.5)
        for b in range(2):
            qb_ref[pl.ds(b * 128, 128), :] = _col_bcast(_tile(q, b)[0:1])

    phase(WM_STEPS, wm_wait, wm_issue, wq_issue, [first_task])
    phase(WQ_STEPS, wq_wait, wq_issue, wo_issue,
          [mod_task(n) for n in range(WM_G)] + [h_task] + [col_task(b, 2) for b in range(0, NC, 2)])
    phase(WO_STEPS, wo_wait, wo_issue, k0_issue, [lambda: q_cols(0)])

    for g in range(NG):
        wg = wo_v[GO - 1, pl.ds(RO - DH + g * 8, 8), :].astype(F32) * vec_ref[V_GA]
        mg = _lane_mean(wg)
        wol_ref[pl.ds(g * 8, 8), pl.ds(0, D)] = wg - mg
        wol_ref[pl.ds(g * 8, 8), pl.ds(D, 128)] = jnp.broadcast_to(mg, (8, 128))

    def scores(h, issue):
        r0 = _mult(_rem(h * DH, 128), 64)

        def kstep(j, carry):
            wait(kbuf.at[j], kvs.at[j])
            issue(j)
            parts = []
            for g in range(NG // 2):
                kg = kbuf[j, pl.ds(g * 16, 16), :].astype(F32)
                for rr in range(2):
                    parts.append(kg[rr * 8:rr * 8 + 8] * qb_ref[pl.ds(r0 + g * 16 + rr * 8, 8), :])
            s_ref[j] = _chain_sum(parts, 4)
            return carry

        lax.fori_loop(0, NB, kstep, 0)

        s = jnp.sum(s_ref[...], axis=1, keepdims=True)
        m = jnp.max(jnp.max(s, axis=0), axis=1, keepdims=True)
        p = jnp.exp(s - m[None])
        l = jnp.sum(jnp.sum(p, axis=0), axis=1, keepdims=True)
        p_ref[...] = jnp.broadcast_to(p, p_ref.shape)
        return 1.0 / l

    def head_body(h, carry):
        inv_l = scores(h, lambda j: kv_issue(v_hbm, vbuf, h, j))
        q_cols(h + 1)

        def vstep(j, acc):
            wait(vbuf.at[j], kvs.at[j])
            kv_issue(k_hbm, kbuf, h + 1, j)
            pj = p_ref[j]
            out = []
            for g in range(NG // 2):
                vg = vbuf[j, pl.ds(g * 16, 16), :].astype(F32)
                for rr in range(2):
                    out.append(acc[2 * g + rr] + vg[rr * 8:rr * 8 + 8] * pj)
            return tuple(out)

        acc = lax.fori_loop(0, NB, vstep, tuple(jnp.zeros((8, 128), F32) for _ in range(NG)))

        hg = _div(h, H // GO)
        r0 = _mult(_rem(h, H // GO) * DH, 8)
        terms = []
        for g in range(NG):
            og = jnp.sum(acc[g], axis=1, keepdims=True) * inv_l
            terms.append(wo_v[hg, pl.ds(r0 + g * 8, 8), :].astype(F32) * og)
        attn_ref[...] += _chain_sum(terms, 2)
        return carry

    lax.fori_loop(0, H - 1, head_body, 0)

    def last_issue(j):
        @pl.when(jnp.logical_and(j < 2 * LN_STEPS, lax.rem(j, 2) == 0))
        def _():
            vlast_issue(lax.div(j, 2))

    inv_l = scores(H - 1, last_issue)

    xp = vec_ref[V_X] + vec_ref[V_GA] * _sub_allreduce(attn_ref[...])
    mp = _lane_mean(xp)
    vec_ref[V_Y] = xp - mp
    vec_ref[V_MISC, :, pl.ds(256, 128)] = jnp.broadcast_to(mp, (8, 128))

    def lstep(j, acc):
        rows = _mult(j * LR, 8)
        wait(vlast.at[pl.ds(rows, LR), :], sems.at[j])

        @pl.when(j < RM // 8)
        def _():
            gb_issue(j)

        for g in range(LR // 8):
            parts = []
            for t in range(NB // 2):
                vg = vlast[pl.ds(rows + g * 8, 8), pl.ds(t * 256, 256)].astype(F32)
                parts += [_tile(vg, cc) * p_ref[2 * t + cc] for cc in range(2)]
            og = jnp.sum(_chain_sum(parts, 4), axis=1, keepdims=True) * inv_l
            acc = acc + wol_ref[pl.ds(rows + g * 8, 8), :] * og
        return acc

    acc = lax.fori_loop(0, LN_STEPS, lstep, jnp.zeros((8, D + 128), F32))

    acc = _sub_allreduce(acc)
    y = vec_ref[V_Y] + acc[:, 0:D]
    m1 = vec_ref[V_MISC, :, pl.ds(256, 128)] + acc[:, D:D + 128]
    st = vec_ref[V_SB]
    yg = y * vec_ref[V_CB]
    r1 = lax.rsqrt(_lane_mean(y * y) + EPS)
    m2 = _lane_mean(yg)
    v2 = _lane_mean(yg * yg) - m2 * m2
    cv = _lane_mean(yg * st)
    r2 = lax.rsqrt(jnp.maximum(r1 * (r1 * v2 + 2.0 * cv) + vec_ref[V_MISC, :, pl.ds(128, 128)], EPS))
    r12 = r1 * r2
    hs = [(_tile(yg, t) - m2) * r12 + _tile(st, t) * r2 for t in range(NT)]

    def tanh_unit(t, r0, n):
        a = w1c[pl.ds(r0, n), :].reshape(n // 8, 8, 128)
        b = b1c[pl.ds(r0, n), :].reshape(n // 8, 8, 128)
        v = hs[t][None] * a + b
        return jnp.tanh(v * (v * v + GELU_KAPPA)).reshape(n, 128)

    def reduce_unit(r0, n, th):
        return jnp.dot(ab_ref[:, pl.ds(r0, n)], th, preferred_element_type=F32, precision=lax.Precision.DEFAULT)

    units = [(t, r0, min(128, FF - NV - r0)) for r0 in range(0, FF - NV, 128) for t in range(NT)]
    n1 = MLP_SPLIT * NT
    acc = [vec_ref[V_MISC, :, pl.ds(0, 128)]] * NT
    held = []
    for k, (t, r0, n) in enumerate(units[:n1]):
        th = tanh_unit(t, r0, n)
        if k < n1 - KS:
            acc[t] = acc[t] + reduce_unit(r0, n, th)
        else:
            held.append(th)
    wait(gb_v, gsem)
    for th, (t, r0, n) in zip(held, units[n1 - KS:n1]):
        acc[t] = acc[t] + reduce_unit(r0, n, th)
    gb = []
    for t, r0, n in units[n1:]:
        acc[t] = acc[t] + reduce_unit(r0, n, tanh_unit(t, r0, n))
        if len(gb) < NT:
            w = gb_v[:, :, pl.ds(len(gb) * 128, 128)].reshape(D, 128)
            gb.append(jnp.dot(sc_ref[...], w, preferred_element_type=F32))
    row = lax.broadcasted_iota(jnp.int32, (8, 128), 0)
    accv = [None] * NT
    for r in range(FF - NV, FF, 8):
        a, b, w = w1c[pl.ds(r, 8), :], b1c[pl.ds(r, 8), :], w2c[pl.ds(r - (FF - 128), 8), :]
        for t in range(NT):
            v = hs[t] * a + b
            g = (v * jnp.tanh(v * (v * v + GELU_KAPPA))) * w
            accv[t] = g if accv[t] is None else accv[t] + g
    outs = []
    for t in range(NT):
        yt = acc[t] * jnp.where(row < 2, hs[t], 1.0) + accv[t]
        outs.append(_tile(y, t) + m1 + gb[t] * _sub_allreduce(yt))
    o_ref[0] = jnp.concatenate(outs, axis=1)[0:1, :].astype(o_ref.dtype)


@jax.jit
def pallas_adaLN_cond__sliding_block_cached__mixer_token_mlp__decode_kernel(
    A_x: jax.Array,
    A_k_cache: jax.Array,
    A_v_cache: jax.Array,
    A_wq: jax.Array,
    A_wo: jax.Array,
    B_x: jax.Array,
    B_w1: jax.Array,
    B_b1: jax.Array,
    B_w2: jax.Array,
    B_b2: jax.Array,
    c: jax.Array,
    w_mod: jax.Array,
):
    del B_x
    kt = jnp.swapaxes(A_k_cache, 2, 3).reshape(H * DH, SK)
    vt = jnp.swapaxes(A_v_cache, 2, 3).reshape(H * DH, SK)
    args = (A_x.reshape(1, D), kt, vt, A_wq.reshape(GM, RM, H * DH), A_wo.reshape(GO, RO, D), B_w1,
            B_b1.reshape(NC, 128), B_w2.reshape(1, FF), B_b2, c, w_mod.reshape(GM, RM, 6 * D))
    scratch = [
        pltpu.VMEM((NB, DH, CB), BF16),
        pltpu.VMEM((NB, DH, CB), BF16),
        pltpu.VMEM((DH, W), BF16),
        pltpu.VMEM((GM, RM, H * DH), BF16),
        pltpu.VMEM((GO, RO, D), BF16),
        pltpu.VMEM((GM, RM, WM_G * D), BF16),
        pltpu.VMEM((GM, RM, D), BF16),
        pltpu.VMEM((1, D), BF16),
        pltpu.VMEM((1, D), BF16),
        pltpu.VMEM((1, FF), BF16),
        pltpu.VMEM((NC, 128), BF16),
        pltpu.VMEM((1, FF), BF16),
        pltpu.VMEM((1,), BF16),
        pltpu.VMEM((256, 128), F32),
        pltpu.VMEM((NB, 8, CB), F32),
        pltpu.VMEM((NB, 8, CB), F32),
        pltpu.VMEM((8, D), F32),
        pltpu.VMEM((9, 8, D), F32),
        pltpu.VMEM((8, D), BF16),
        pltpu.VMEM((8, D), BF16),
        pltpu.VMEM((FF, 128), F32),
        pltpu.VMEM((FF, 128), F32),
        pltpu.VMEM((128, 128), F32),
        pltpu.VMEM((8, FF), F32),
        pltpu.VMEM((DH, D + 128), F32),
        pltpu.SemaphoreType.DMA((NS,)),
        pltpu.SemaphoreType.DMA((NB,)),
        pltpu.SemaphoreType.DMA((6,)),
        pltpu.SemaphoreType.DMA(()),
    ]
    return pl.pallas_call(
        _kernel,
        in_specs=[pl.BlockSpec(memory_space=pl.ANY)] * len(args),
        out_specs=pl.BlockSpec(memory_space=pltpu.VMEM),
        out_shape=jax.ShapeDtypeStruct((1, 1, D), BF16),
        scratch_shapes=scratch,
        compiler_params=pltpu.CompilerParams(
            vmem_limit_bytes=120 * 1024 * 1024,
            disable_bounds_checks=True,
            disable_semaphore_checks=True,
        ),
    )(*args)
```

```python
import functools

import jax
import jax.numpy as jnp
from jax import lax
import jax.experimental.pallas as pl
import jax.experimental.pallas.tpu as pltpu

F32 = jnp.float32
BF16 = jnp.bfloat16

D = 640
H = 32
DH = 192
SK = 32768
W = 4096
FF = 1536
EPS = 1e-5
NT = D // 128
NC = FF // 128
NG = DH // 8

CB = 128
NB = W // CB
HR = 16

NS = 16
GM = 10
RM = D // GM
GO = 8
RO = H * DH // GO
GH = 2
WM_G = 5
WM_STEPS = WM_G * (RM // 8)
WQ_C = 384
WQ_STEPS = (H * DH // WQ_C) * (RM // 8)
WO_STEPS = RO // 8
SEG = 4

DR = 64
ND = 2
DG = ND * DR // 8
assert DG == NS
SPV = 64

MLP_SPLIT = 55
KS = 5
NV = 96

GELU_K0 = 0.7978845608028654
GELU_K1 = GELU_K0 * 0.044715
GELU_S = GELU_K1 ** (1.0 / 3.0)
GELU_KAPPA = GELU_K0 / GELU_S

V_X, V_XN, V_SA, V_CA, V_GA, V_SB, V_CB, V_Y, V_MISC = range(9)


def _lane_mean(v):
    return jnp.sum(v, axis=-1, keepdims=True) * (1.0 / D)


def _col_bcast(row):
    return jnp.broadcast_to(row, (128, 128)).T


def _chain_sum(xs, n):
    chains = [functools.reduce(lambda a, b: a + b, xs[i::n]) for i in range(n)]
    while len(chains) > 1:
        chains = [chains[i] + chains[i + 1] for i in range(0, len(chains), 2)]
    return chains[0]


def _sub_allreduce(v):
    v = v + pltpu.roll(v, 4, 0)
    v = v + pltpu.roll(v, 2, 0)
    return v + pltpu.roll(v, 1, 0)


def _tile(v, t):
    return v[:, t * 128:(t + 1) * 128]


def _mult(i, n):
    return i if isinstance(i, int) else pl.multiple_of(i, n)


def _rem(i, n):
    return i % n if isinstance(i, int) else lax.rem(i, n)


def _div(i, n):
    return i // n if isinstance(i, int) else lax.div(i, n)


def _kernel(x_hbm, k_hbm, v_hbm, wq_hbm, wo_hbm, w1_hbm, b1_hbm, w2_hbm, b2_hbm, c_hbm, wm_hbm,
            o_ref,
            kbuf, vbuf, wq_v, wo_v, wm_v, gb_v, x_v, c_v, w1_v, b1_v, w2_v, b2_v,
            qb_ref, s_ref, p_ref, attn_ref, vec_ref, sc_ref, h8_ref, w1c, b1c, w2c, ab_ref,
            sems, kvs, ssems, gsem):

    def dma(src, dst, sem, prio):
        pltpu.make_async_copy(src, dst, sem).start(priority=prio)

    def wait(dst, sem):
        pltpu.make_async_copy(dst, dst, sem).wait()

    def weight_steps(hbm, vmem, groups, ncols, ncb, base):
        def where(i):
            if ncb == 1:
                return pl.ds(_mult(i * 8, 8), 8), pl.ds(0, ncols)
            return pl.ds(_mult(_div(i, ncb) * 8, 8), 8), pl.ds(_mult(_rem(i, ncb) * ncols, 128), ncols)

        def issue(i, which=(0, 1)):
            r, c = where(i)
            sem = sems.at[_rem(i + base, NS)]
            hi, lo = pl.ds(0, GH), pl.ds(GH, groups - GH)
            if 0 in which:
                dma(hbm.at[hi, r, c], vmem.at[hi, r, c], sem, 0)
            if 1 in which:
                dma(hbm.at[lo, r, c], vmem.at[lo, r, c], sem, 1)

        def wait_(i):
            r, c = where(i)
            wait(vmem.at[pl.ds(0, groups), r, c], sems.at[_rem(i + base, NS)])

        return issue, wait_

    wm_issue, wm_wait = weight_steps(wm_hbm, wm_v, GM, D, WM_G, 0)
    wq_issue, wq_wait = weight_steps(wq_hbm, wq_v, GM, WQ_C, H * DH // WQ_C, WM_STEPS % NS)
    wo_issue, wo_wait = weight_steps(wo_hbm, wo_v, GO, D, 1, (WM_STEPS + WQ_STEPS) % NS)

    wo7_issue, wo7_wait = weight_steps(wo_hbm, wo_v, GO - 1, D, 1, (WM_STEPS + WQ_STEPS) % NS)

    def kv_issue(src, buf, h, j):
        c = pl.ds(_mult(SK - W + j * CB, 128), CB)
        dma(src.at[pl.ds(_mult(h * DH, 8), HR), c], buf.at[j, pl.ds(0, HR), :], kvs.at[j], 0)
        dma(src.at[pl.ds(_mult(h * DH + HR, 8), DH - HR), c], buf.at[j, pl.ds(HR, DH - HR), :], kvs.at[j], 1)

    def k0_issue(j):
        for u in range(NB // NS):
            kv_issue(k_hbm, kbuf, 0, j * (NB // NS) + u)

    def end_issue(j):
        @pl.when(j < ND)
        def _():
            r = pl.ds(pl.multiple_of(RO - ND * DR + j * DR, 8), DR)
            dma(wo_hbm.at[GO - 1, r, :], wo_v.at[GO - 1, r, :], sems.at[j], 1)

        @pl.when(j == ND)
        def _():
            for r in range(0, RM, 8):
                dma(wm_hbm.at[:, pl.ds(r, 8), pl.ds(WM_G * D, D)], gb_v.at[:, pl.ds(r, 8), :], gsem, 1)

    def pump(lo, hi, wait_fn, issue_fn, off):
        def body(i, carry):
            wait_fn(i)
            issue_fn(i + off)
            return carry
        lax.fori_loop(lo, hi, body, 0)

    def phase(n, wait_fn, issue_fn, next_issue, tasks):
        for k, task in enumerate(tasks):
            pump(k * SEG, (k + 1) * SEG, wait_fn, issue_fn, NS)
            task()
        pump(len(tasks) * SEG, n - NS, wait_fn, issue_fn, NS)
        pump(n - NS, n, wait_fn, next_issue, NS - n)

    for i in range(NS):
        wm_issue(i, (1,))
    small = [pltpu.make_async_copy(s, d, ssems.at[n]) for n, (s, d) in enumerate(
        [(c_hbm, c_v), (x_hbm, x_v), (w1_hbm, w1_v), (b1_hbm, b1_v), (w2_hbm, w2_v), (b2_hbm, b2_v)])]
    for cp in small:
        cp.start()

    def spaced(i, carry):
        wm_issue(i, (0,))
        w1c[pl.ds(0, SPV * 8), :] = jnp.full((SPV * 8, 128), i, jnp.int32).astype(F32)
        return carry

    lax.fori_loop(0, NS, spaced, 0)

    def first_task():
        for cp in small:
            cp.wait()
        c = c_v[...].astype(F32)
        sc_ref[...] = jnp.broadcast_to(c * jax.nn.sigmoid(c), (8, D)).astype(BF16)
        x8 = jnp.broadcast_to(x_v[...].astype(F32), (8, D))
        xc = x8 - _lane_mean(x8)
        vec_ref[V_X] = x8
        vec_ref[V_XN] = xc * lax.rsqrt(_lane_mean(xc * xc) + EPS)
        attn_ref[...] = jnp.zeros(attn_ref.shape, F32)
        w2f = w2_v[...].astype(F32) * 0.5
        w1r = w1_v[...].astype(F32)
        b1r = b1_v[...].astype(F32)
        row = lax.broadcasted_iota(jnp.int32, (8, 128), 0)
        sum_ab = jnp.zeros((8, 128), F32)
        for b in range(NC):
            wa = _tile(w2f, b) * _tile(w1r, b)
            wb = _tile(w2f, b) * b1r[b:b + 1, :]
            ab = jnp.where(row < 2, jnp.broadcast_to(wa, (8, 128)), jnp.broadcast_to(wb, (8, 128)))
            ab = jnp.where(row < 4, ab, 0.0)
            hi = ab.astype(BF16).astype(F32)
            ab_ref[:, pl.ds(b * 128, 128)] = jnp.where(row % 2 == 0, hi, (ab - hi).astype(BF16).astype(F32))
            sum_ab = sum_ab + jnp.where(row % 2 == 0, ab, 0.0)
        sum_ab = jnp.broadcast_to(jnp.sum(sum_ab, axis=1, keepdims=True), (8, 128))
        b2 = jnp.broadcast_to(b2_v[...].astype(F32), (8, 128))
        vec_ref[V_MISC, :, pl.ds(0, 128)] = sum_ab + jnp.where(row == 2, b2, 0.0)

    def col_task(b0, nb):
        def task():
            w1f = w1_v[...].astype(F32) * GELU_S
            b1f = b1_v[...].astype(F32) * GELU_S
            for b in range(b0, b0 + nb):
                w1c[pl.ds(b * 128, 128), :] = _col_bcast(_tile(w1f, b))
                b1c[pl.ds(b * 128, 128), :] = _col_bcast(b1f[b:b + 1, :])
            if b0 == 0:
                w2c[...] = _col_bcast(_tile(w2_v[...].astype(F32) * (0.5 / GELU_S), NC - 1))
        return task

    def mod_task(n):
        def task():
            w = wm_v[:, :, pl.ds(n * D, D)].reshape(D, D)
            vec_ref[V_SA + n] = jnp.dot(sc_ref[...], w, preferred_element_type=F32)
        return task

    def h_task():
        h8_ref[...] = (vec_ref[V_XN] * (1.0 + vec_ref[V_CA]) + vec_ref[V_SA]).astype(BF16)
        sb = vec_ref[V_SB]
        st = sb - _lane_mean(sb)
        vec_ref[V_SB] = st
        g = 1.0 + vec_ref[V_CB]
        vec_ref[V_CB] = g
        vec_ref[V_MISC, :, pl.ds(256, 128)] = jnp.broadcast_to(_lane_mean(g), (8, 128))
        vec_ref[V_MISC, :, pl.ds(384, 128)] = jnp.broadcast_to(_lane_mean(g * g), (8, 128))
        vec_ref[V_MISC, :, pl.ds(512, 128)] = jnp.broadcast_to(_lane_mean(g * st), (8, 128))
        vec_ref[V_MISC, :, pl.ds(128, 128)] = jnp.broadcast_to(_lane_mean(st * st) + EPS, (8, 128))

    def q_cols(h):
        c0 = _mult(_div(h * DH, 128) * 128, 128)
        q = jnp.dot(h8_ref[...], wq_v[:, :, pl.ds(c0, 256)].reshape(D, 256), preferred_element_type=F32)
        q = q.astype(BF16).astype(F32) * (DH ** -0.5)
        for b in range(2):
            qb_ref[pl.ds(b * 128, 128), :] = _col_bcast(_tile(q, b)[0:1])

    phase(WM_STEPS, wm_wait, wm_issue, wq_issue, [first_task])
    phase(WQ_STEPS, wq_wait, wq_issue, wo_issue,
          [mod_task(n) for n in range(WM_G)] + [h_task] + [col_task(b, 2) for b in range(0, NC, 2)])
    phase(WO_STEPS - DG, wo_wait, wo_issue, lambda i: wo7_issue(i + WO_STEPS - DG), [lambda: q_cols(0)])
    pump(WO_STEPS - DG, WO_STEPS, wo7_wait, k0_issue, DG - WO_STEPS)

    def scores(h, issue):
        r0 = _mult(_rem(h * DH, 128), 64)

        def kstep(j, carry):
            wait(kbuf.at[j], kvs.at[j])
            issue(j)
            parts = []
            for g in range(NG // 2):
                kg = kbuf[j, pl.ds(g * 16, 16), :].astype(F32)
                for rr in range(2):
                    parts.append(kg[rr * 8:rr * 8 + 8] * qb_ref[pl.ds(r0 + g * 16 + rr * 8, 8), :])
            s_ref[j] = _chain_sum(parts, 4)
            return carry

        lax.fori_loop(0, NB, kstep, 0)

        s = jnp.sum(s_ref[...], axis=1, keepdims=True)
        m = jnp.max(jnp.max(s, axis=0), axis=1, keepdims=True)
        p = jnp.exp(s - m[None])
        l = jnp.sum(jnp.sum(p, axis=0), axis=1, keepdims=True)
        p_ref[...] = jnp.broadcast_to(p, p_ref.shape)
        return 1.0 / l

    def values(issue):
        def vstep(j, acc):
            wait(vbuf.at[j], kvs.at[j])
            issue(j)
            pj = p_ref[j]
            out = []
            for g in range(NG // 2):
                vg = vbuf[j, pl.ds(g * 16, 16), :].astype(F32)
                for rr in range(2):
                    out.append(acc[2 * g + rr] + vg[rr * 8:rr * 8 + 8] * pj)
            return tuple(out)

        return lax.fori_loop(0, NB, vstep, tuple(jnp.zeros((8, 128), F32) for _ in range(NG)))

    def project(hg, r0, og):
        return _chain_sum([wo_v[hg, pl.ds(r0 + g * 8, 8), :].astype(F32) * o for g, o in enumerate(og)], 2)

    def head_body(h, carry):
        inv_l = scores(h, lambda j: kv_issue(v_hbm, vbuf, h, j))
        q_cols(h + 1)
        acc = values(lambda j: kv_issue(k_hbm, kbuf, h + 1, j))
        hg = _div(h, H // GO)
        r0 = _mult(_rem(h, H // GO) * DH, 8)
        og = [jnp.sum(a, axis=1, keepdims=True) * inv_l for a in acc]
        attn_ref[...] += project(hg, r0, og)
        return carry

    lax.fori_loop(0, H - 1, head_body, 0)

    inv_l = scores(H - 1, lambda j: kv_issue(v_hbm, vbuf, H - 1, j))
    xp = vec_ref[V_X] + vec_ref[V_GA] * _sub_allreduce(attn_ref[...])
    mp = _lane_mean(xp)
    vec_ref[V_Y] = xp - mp
    vec_ref[V_X, :, pl.ds(0, 128)] = jnp.broadcast_to(mp, (8, 128))
    acc = values(end_issue)
    og = [jnp.sum(a, axis=1, keepdims=True) * inv_l for a in acc]
    for g in range(DG):
        s_ref[g] = jnp.broadcast_to(og[NG - DG + g], (8, 128))
    part = project(GO - 1, RO - DH, og[:NG - DG])

    def dstep(i, part):
        r = pl.multiple_of(RO - ND * DR + i * DR, 8)
        wait(wo_v.at[GO - 1, pl.ds(r, DR), :], sems.at[i])
        terms = []
        for g in range(DR // 8):
            w = wo_v[GO - 1, pl.ds(r + g * 8, 8), :].astype(F32)
            o = s_ref[i * (DR // 8) + g]
            terms.append(jnp.concatenate([_tile(w, t) * o for t in range(NT)], axis=1))
        return part + _chain_sum(terms, 2)

    part = lax.fori_loop(0, ND, dstep, part)

    y = vec_ref[V_Y] + vec_ref[V_GA] * _sub_allreduce(part)
    m1 = vec_ref[V_X, :, pl.ds(0, 128)]
    st = vec_ref[V_SB]
    g = vec_ref[V_CB]
    yg = y * g
    a0, a1, a2 = _lane_mean(y), _lane_mean(y * y), _lane_mean(yg)
    a3, a4, a5 = _lane_mean(yg * yg), _lane_mean(yg * g), _lane_mean(yg * st)
    g1, g2, gs = (vec_ref[V_MISC, :, pl.ds(c, 128)] for c in (256, 384, 512))
    r1 = lax.rsqrt(jnp.maximum(a1 - a0 * a0 + EPS, EPS))
    m2 = a2 - a0 * g1
    v2 = a3 - a0 * (2.0 * a4 - a0 * g2) - m2 * m2
    cv = a5 - a0 * gs
    r2 = lax.rsqrt(jnp.maximum(r1 * (r1 * v2 + 2.0 * cv) + vec_ref[V_MISC, :, pl.ds(128, 128)], EPS))
    r12 = r1 * r2
    hs = [(_tile(yg, t) - (_tile(g, t) * a0 + m2)) * r12 + _tile(st, t) * r2 for t in range(NT)]

    def tanh_unit(t, r0, n):
        a = w1c[pl.ds(r0, n), :].reshape(n // 8, 8, 128)
        b = b1c[pl.ds(r0, n), :].reshape(n // 8, 8, 128)
        v = hs[t][None] * a + b
        return jnp.tanh(v * (v * v + GELU_KAPPA)).reshape(n, 128)

    def reduce_unit(r0, n, th):
        return jnp.dot(ab_ref[:, pl.ds(r0, n)], th, preferred_element_type=F32, precision=lax.Precision.DEFAULT)

    units = [(t, r0, min(128, FF - NV - r0)) for r0 in range(0, FF - NV, 128) for t in range(NT)]
    acc = [vec_ref[V_MISC, :, pl.ds(0, 128)]] * NT
    for k, (t, r0, n) in enumerate(units[:MLP_SPLIT]):
        th = tanh_unit(t, r0, n)
        if k < MLP_SPLIT - KS:
            acc[t] = acc[t] + reduce_unit(r0, n, th)
        else:
            qb_ref[pl.ds((k - (MLP_SPLIT - KS)) * 128, n), :] = th
    wait(gb_v, gsem)
    for k, (t, r0, n) in enumerate(units[MLP_SPLIT - KS:MLP_SPLIT]):
        acc[t] = acc[t] + reduce_unit(r0, n, qb_ref[pl.ds(k * 128, n), :])
    gb = []
    for t, r0, n in units[MLP_SPLIT:]:
        acc[t] = acc[t] + reduce_unit(r0, n, tanh_unit(t, r0, n))
        w = gb_v[:, :, pl.ds(len(gb) * 128, 128)].reshape(D, 128)
        gb.append(jnp.dot(sc_ref[...], w, preferred_element_type=F32))
    row = lax.broadcasted_iota(jnp.int32, (8, 128), 0)
    accv = [None] * NT
    for r in range(FF - NV, FF, 8):
        a, b, w = w1c[pl.ds(r, 8), :], b1c[pl.ds(r, 8), :], w2c[pl.ds(r - (FF - 128), 8), :]
        for t in range(NT):
            v = hs[t] * a + b
            g = (v * jnp.tanh(v * (v * v + GELU_KAPPA))) * w
            accv[t] = g if accv[t] is None else accv[t] + g
    outs = []
    for t in range(NT):
        yt = acc[t] * jnp.where(row < 2, hs[t], 1.0) + accv[t]
        outs.append(_tile(y, t) + m1 + gb[t] * _sub_allreduce(yt))
    o_ref[0] = jnp.concatenate(outs, axis=1)[0:1, :].astype(o_ref.dtype)


@jax.jit
def pallas_adaLN_cond__sliding_block_cached__mixer_token_mlp__decode_kernel(
    A_x: jax.Array,
    A_k_cache: jax.Array,
    A_v_cache: jax.Array,
    A_wq: jax.Array,
    A_wo: jax.Array,
    B_x: jax.Array,
    B_w1: jax.Array,
    B_b1: jax.Array,
    B_w2: jax.Array,
    B_b2: jax.Array,
    c: jax.Array,
    w_mod: jax.Array,
):
    del B_x
    kt = jnp.swapaxes(A_k_cache, 2, 3).reshape(H * DH, SK)
    vt = jnp.swapaxes(A_v_cache, 2, 3).reshape(H * DH, SK)
    args = (A_x.reshape(1, D), kt, vt, A_wq.reshape(GM, RM, H * DH), A_wo.reshape(GO, RO, D), B_w1,
            B_b1.reshape(NC, 128), B_w2.reshape(1, FF), B_b2, c, w_mod.reshape(GM, RM, 6 * D))
    scratch = [
        pltpu.VMEM((NB, DH, CB), BF16),
        pltpu.VMEM((NB, DH, CB), BF16),
        pltpu.VMEM((GM, RM, H * DH), BF16),
        pltpu.VMEM((GO, RO, D), BF16),
        pltpu.VMEM((GM, RM, WM_G * D), BF16),
        pltpu.VMEM((GM, RM, D), BF16),
        pltpu.VMEM((1, D), BF16),
        pltpu.VMEM((1, D), BF16),
        pltpu.VMEM((1, FF), BF16),
        pltpu.VMEM((NC, 128), BF16),
        pltpu.VMEM((1, FF), BF16),
        pltpu.VMEM((1,), BF16),
        pltpu.VMEM((KS * 128, 128), F32),
        pltpu.VMEM((NB, 8, CB), F32),
        pltpu.VMEM((NB, 8, CB), F32),
        pltpu.VMEM((8, D), F32),
        pltpu.VMEM((9, 8, D), F32),
        pltpu.VMEM((8, D), BF16),
        pltpu.VMEM((8, D), BF16),
        pltpu.VMEM((FF, 128), F32),
        pltpu.VMEM((FF, 128), F32),
        pltpu.VMEM((128, 128), F32),
        pltpu.VMEM((8, FF), F32),
        pltpu.SemaphoreType.DMA((NS,)),
        pltpu.SemaphoreType.DMA((NB,)),
        pltpu.SemaphoreType.DMA((6,)),
        pltpu.SemaphoreType.DMA(()),
    ]
    return pl.pallas_call(
        _kernel,
        in_specs=[pl.BlockSpec(memory_space=pl.ANY)] * len(args),
        out_specs=pl.BlockSpec(memory_space=pltpu.VMEM),
        out_shape=jax.ShapeDtypeStruct((1, 1, D), BF16),
        scratch_shapes=scratch,
        compiler_params=pltpu.CompilerParams(
            vmem_limit_bytes=120 * 1024 * 1024,
            disable_bounds_checks=True,
            disable_semaphore_checks=True,
        ),
    )(*args)
```

```python
import functools

import jax
import jax.numpy as jnp
from jax import lax
import jax.experimental.pallas as pl
import jax.experimental.pallas.tpu as pltpu

F32 = jnp.float32
BF16 = jnp.bfloat16

D = 640
H = 32
DH = 192
SK = 32768
W = 4096
FF = 1536
EPS = 1e-5
NT = D // 128
NC = FF // 128
NG = DH // 8

CB = 128
NB = W // CB
HR = 16

NS = 16
GM = 10
RM = D // GM
GH = 2
WM_G = 5
WM_STEPS = WM_G * (RM // 8)
GF = 15
RF = D * H * DH // (128 * GF)
F_STEPS = RF // 8
SEG = 4
SEGF = 14

DR = 64
ND = 2
DG = ND * DR // 8
SPV = 64

MLP_SPLIT = 55
KS = 5
NV = 96

GELU_K0 = 0.7978845608028654
GELU_K1 = GELU_K0 * 0.044715
GELU_S = GELU_K1 ** (1.0 / 3.0)
GELU_KAPPA = GELU_K0 / GELU_S

V_X, V_XN, V_SA, V_CA, V_GA, V_SB, V_CB, V_Y, V_MISC = range(9)


def _lane_mean(v):
    return jnp.sum(v, axis=-1, keepdims=True) * (1.0 / D)


def _col_bcast(row):
    return jnp.broadcast_to(row, (128, 128)).T


def _chain_sum(xs, n):
    chains = [functools.reduce(lambda a, b: a + b, xs[i::n]) for i in range(n)]
    while len(chains) > 1:
        chains = [chains[i] + chains[i + 1] for i in range(0, len(chains), 2)]
    return chains[0]


def _sub_allreduce(v):
    v = v + pltpu.roll(v, 4, 0)
    v = v + pltpu.roll(v, 2, 0)
    return v + pltpu.roll(v, 1, 0)


def _tile(v, t):
    return v[:, t * 128:(t + 1) * 128]


def _mult(i, n):
    return i if isinstance(i, int) else pl.multiple_of(i, n)


def _rem(i, n):
    if isinstance(i, int):
        return i % n
    return i & (n - 1) if n & (n - 1) == 0 else lax.rem(i, n)


def _div(i, n):
    if isinstance(i, int):
        return i // n
    return i >> (n.bit_length() - 1) if n & (n - 1) == 0 else lax.div(i, n)


def _kernel(x_hbm, k_hbm, v_hbm, wq_hbm, wo_hbm, w1_hbm, b1_hbm, w2_hbm, b2_hbm, c_hbm, wm_hbm,
            o_ref,
            kbuf, vbuf, wq_v, wo_v, wm_v, gb_v, x_v, c_v, w1_v, b1_v, w2_v, b2_v,
            qb_ref, s_ref, p_ref, attn_ref, vec_ref, sc_ref, h8_ref, w1c, b1c, w2c, ab_ref,
            sems, kvs, ssems, gsem):

    def dma(src, dst, sem, prio):
        pltpu.make_async_copy(src, dst, sem).start(priority=prio)

    def wait(dst, sem):
        pltpu.make_async_copy(dst, dst, sem).wait()

    def steps(hbm, vmem, groups, where, sem):
        def issue(i, which=(0, 1)):
            idx = where(i)
            for g, prio in ((pl.ds(0, GH), 0), (pl.ds(GH, groups - GH), 1)):
                if prio in which:
                    dma(hbm.at[(g,) + idx], vmem.at[(g,) + idx], sem(i), prio)

        def wait_(i):
            wait(vmem.at[(pl.ds(0, groups),) + where(i)], sem(i))

        return issue, wait_

    wm_issue, wm_wait = steps(
        wm_hbm, wm_v, GM,
        lambda i: (pl.ds(_mult(_div(i, WM_G) * 8, 8), 8), pl.ds(_mult(_rem(i, WM_G) * D, 128), D)),
        lambda i: sems.at[_rem(i, NS)])

    def flat_steps(hbm, vmem, groups):
        return steps(hbm, vmem, groups, lambda i: (pl.ds(_mult(i * 8, 8), 8), slice(None)),
                     lambda i: kvs.at[_rem(i, NB)])

    wq_issue, wq_wait = flat_steps(wq_hbm, wq_v, GF)
    wo_issue, wo_wait = flat_steps(wo_hbm, wo_v, GF)
    wos_issue, wos_wait = flat_steps(wo_hbm, wo_v, GF - 1)
    wq_t = wq_v.reshape(D // 8, H * DH // 16, 128)
    wo_t = wo_v.reshape(GF * RF, 128)

    def kv_issue(src, buf, h, j):
        c = pl.ds(_mult(SK - W + j * CB, 128), CB)
        dma(src.at[pl.ds(_mult(h * DH, 8), HR), c], buf.at[j, pl.ds(0, HR), :], kvs.at[j], 0)
        dma(src.at[pl.ds(_mult(h * DH + HR, 8), DH - HR), c], buf.at[j, pl.ds(HR, DH - HR), :], kvs.at[j], 1)

    def wq0_issue(j):
        for u in range(NB // NS):
            wq_issue(j * (NB // NS) + u)

    def end_issue(j):
        @pl.when(j < ND)
        def _():
            r = pl.ds(pl.multiple_of(RF - (ND - j) * DR * NT, 8), DR * NT)
            dma(wo_hbm.at[GF - 1, r, :], wo_v.at[GF - 1, r, :], sems.at[j], 1)

        @pl.when(j == ND)
        def _():
            for r in range(0, RM, 8):
                dma(wm_hbm.at[:, pl.ds(r, 8), pl.ds(WM_G * D, D)], gb_v.at[:, pl.ds(r, 8), :], gsem, 1)

    def pump(lo, hi, wait_fn, issue_fn, off):
        def body(i, carry):
            wait_fn(i)
            issue_fn(i + off)
            return carry
        lax.fori_loop(lo, hi, body, 0)

    def phase(n, wait_fn, issue_fn, next_issue, tasks, win, seg):
        for k, task in enumerate(tasks):
            pump(k * seg, (k + 1) * seg, wait_fn, issue_fn, win)
            task()
        pump(len(tasks) * seg, n - win, wait_fn, issue_fn, win)
        pump(n - win, n, wait_fn, next_issue, win - n)

    for i in range(NS):
        wm_issue(i, (1,))
    small = [pltpu.make_async_copy(s, d, ssems.at[n]) for n, (s, d) in enumerate(
        [(c_hbm, c_v), (x_hbm, x_v), (w1_hbm, w1_v), (b1_hbm, b1_v), (w2_hbm, w2_v), (b2_hbm, b2_v)])]
    for cp in small:
        cp.start()

    def spaced(i, carry):
        wm_issue(i, (0,))
        w1c[pl.ds(0, SPV * 8), :] = jnp.full((SPV * 8, 128), i, jnp.int32).astype(F32)
        return carry

    lax.fori_loop(0, NS, spaced, 0)

    def first_task():
        for cp in small:
            cp.wait()
        c = c_v[...].astype(F32)
        sc_ref[...] = jnp.broadcast_to(c * jax.nn.sigmoid(c), (8, D)).astype(BF16)
        x8 = jnp.broadcast_to(x_v[...].astype(F32), (8, D))
        xc = x8 - _lane_mean(x8)
        vec_ref[V_X] = x8
        vec_ref[V_XN] = xc * lax.rsqrt(_lane_mean(xc * xc) + EPS)
        attn_ref[...] = jnp.zeros(attn_ref.shape, F32)
        w2f = w2_v[...].astype(F32) * 0.5
        w1r = w1_v[...].astype(F32)
        b1r = b1_v[...].astype(F32)
        row = lax.broadcasted_iota(jnp.int32, (8, 128), 0)
        sum_ab = jnp.zeros((8, 128), F32)
        for b in range(NC):
            wa = _tile(w2f, b) * _tile(w1r, b)
            wb = _tile(w2f, b) * b1r[b:b + 1, :]
            ab = jnp.where(row < 2, jnp.broadcast_to(wa, (8, 128)), jnp.broadcast_to(wb, (8, 128)))
            ab = jnp.where(row < 4, ab, 0.0)
            hi = ab.astype(BF16).astype(F32)
            ab_ref[:, pl.ds(b * 128, 128)] = jnp.where(row % 2 == 0, hi, (ab - hi).astype(BF16).astype(F32))
            sum_ab = sum_ab + jnp.where(row % 2 == 0, ab, 0.0)
        sum_ab = jnp.broadcast_to(jnp.sum(sum_ab, axis=1, keepdims=True), (8, 128))
        b2 = jnp.broadcast_to(b2_v[...].astype(F32), (8, 128))
        vec_ref[V_MISC, :, pl.ds(0, 128)] = sum_ab + jnp.where(row == 2, b2, 0.0)

    def col_task(b0, nb):
        def task():
            w1f = w1_v[...].astype(F32) * GELU_S
            b1f = b1_v[...].astype(F32) * GELU_S
            for b in range(b0, b0 + nb):
                w1c[pl.ds(b * 128, 128), :] = _col_bcast(_tile(w1f, b))
                b1c[pl.ds(b * 128, 128), :] = _col_bcast(b1f[b:b + 1, :])
            if b0 == 0:
                w2c[...] = _col_bcast(_tile(w2_v[...].astype(F32) * (0.5 / GELU_S), NC - 1))
        return task

    def mod_task(n):
        def task():
            w = wm_v[:, :, pl.ds(n * D, D)].reshape(D, D)
            vec_ref[V_SA + n] = jnp.dot(sc_ref[...], w, preferred_element_type=F32)
        return task

    def h_task():
        h8_ref[...] = (vec_ref[V_XN] * (1.0 + vec_ref[V_CA]) + vec_ref[V_SA]).astype(BF16)
        sb = vec_ref[V_SB]
        st = sb - _lane_mean(sb)
        vec_ref[V_SB] = st
        g = 1.0 + vec_ref[V_CB]
        vec_ref[V_CB] = g
        vec_ref[V_MISC, :, pl.ds(256, 128)] = jnp.broadcast_to(_lane_mean(g), (8, 128))
        vec_ref[V_MISC, :, pl.ds(384, 128)] = jnp.broadcast_to(_lane_mean(g * g), (8, 128))
        vec_ref[V_MISC, :, pl.ds(512, 128)] = jnp.broadcast_to(_lane_mean(g * st), (8, 128))
        vec_ref[V_MISC, :, pl.ds(128, 128)] = jnp.broadcast_to(_lane_mean(st * st) + EPS, (8, 128))

    def q_cols(h):
        c0 = _div(h * DH, 128)
        for b in range(2):
            w = wq_t[:, pl.ds(_mult((c0 + b) * 8, 8), 8), :].reshape(D, 128)
            q = jnp.dot(h8_ref[...], w, preferred_element_type=F32)
            q = q.astype(BF16).astype(F32) * (DH ** -0.5)
            qb_ref[pl.ds(b * 128, 128), :] = _col_bcast(q[0:1])

    phase(WM_STEPS, wm_wait, wm_issue, wq0_issue, [first_task], NS, SEG)
    phase(F_STEPS, wq_wait, wq_issue, wo_issue,
          [mod_task(n) for n in range(WM_G)] + [h_task] + [col_task(b, 2) for b in range(0, NC, 2)], NB, SEGF)
    nfull = F_STEPS - DG * NT
    phase(nfull, wo_wait, wo_issue, lambda i: wos_issue(i + nfull), [lambda: q_cols(0)], NB, SEGF)
    pump(nfull, F_STEPS - NB, wos_wait, wos_issue, NB)
    pump(F_STEPS - NB, F_STEPS, wos_wait, lambda j: kv_issue(k_hbm, kbuf, 0, j), NB - F_STEPS)

    def scores(h, issue):
        r0 = _mult(_rem(h * DH, 128), 64)

        def kstep(j, carry):
            wait(kbuf.at[j], kvs.at[j])
            issue(j)
            parts = []
            for g in range(NG // 2):
                kg = kbuf[j, pl.ds(g * 16, 16), :].astype(F32)
                for rr in range(2):
                    parts.append(kg[rr * 8:rr * 8 + 8] * qb_ref[pl.ds(r0 + g * 16 + rr * 8, 8), :])
            s_ref[j] = _chain_sum(parts, 4)
            return carry

        lax.fori_loop(0, NB, kstep, 0)

        s = jnp.sum(s_ref[...], axis=1, keepdims=True)
        m = jnp.max(jnp.max(s, axis=0), axis=1, keepdims=True)
        p = jnp.exp(s - m[None])
        l = jnp.sum(jnp.sum(p, axis=0), axis=1, keepdims=True)
        p_ref[...] = jnp.broadcast_to(p, p_ref.shape)
        return 1.0 / l

    def values(issue):
        def vstep(j, acc):
            wait(vbuf.at[j], kvs.at[j])
            issue(j)
            pj = p_ref[j]
            out = []
            for g in range(NG // 2):
                vg = vbuf[j, pl.ds(g * 16, 16), :].astype(F32)
                for rr in range(2):
                    out.append(acc[2 * g + rr] + vg[rr * 8:rr * 8 + 8] * pj)
            return tuple(out)

        return lax.fori_loop(0, NB, vstep, tuple(jnp.zeros((8, 128), F32) for _ in range(NG)))

    def project(rt0, og):
        terms = [[] for _ in range(NT)]
        for k in range(len(og) * NT // 2):
            w = wo_t[pl.ds(_mult(rt0 * NT * 8 + k * 16, 16), 16), :].astype(F32)
            for u in (2 * k, 2 * k + 1):
                terms[u % NT].append(w[(u % 2) * 8:(u % 2) * 8 + 8] * og[u // NT])
        return jnp.concatenate([_chain_sum(ts, 2) for ts in terms], axis=1)

    def head_body(h, carry):
        inv_l = scores(h, lambda j: kv_issue(v_hbm, vbuf, h, j))
        q_cols(h + 1)
        acc = values(lambda j: kv_issue(k_hbm, kbuf, h + 1, j))
        og = [jnp.sum(a, axis=1, keepdims=True) * inv_l for a in acc]
        attn_ref[...] += project(h * NG, og)
        return carry

    lax.fori_loop(0, H - 1, head_body, 0)

    inv_l = scores(H - 1, lambda j: kv_issue(v_hbm, vbuf, H - 1, j))
    xp = vec_ref[V_X] + vec_ref[V_GA] * _sub_allreduce(attn_ref[...])
    mp = _lane_mean(xp)
    vec_ref[V_Y] = xp - mp
    vec_ref[V_X, :, pl.ds(0, 128)] = jnp.broadcast_to(mp, (8, 128))
    acc = values(end_issue)
    og = [jnp.sum(a, axis=1, keepdims=True) * inv_l for a in acc]
    for g in range(DG):
        s_ref[g] = jnp.broadcast_to(og[NG - DG + g], (8, 128))
    part = project((H - 1) * NG, og[:NG - DG])

    def dstep(i, part):
        r = pl.ds(pl.multiple_of(RF - (ND - i) * DR * NT, 8), DR * NT)
        wait(wo_v.at[GF - 1, r, :], sems.at[i])
        g0 = i * (DR // 8)
        return part + project(H * NG - DG + g0, [s_ref[g0 + g] for g in range(DR // 8)])

    part = lax.fori_loop(0, ND, dstep, part)

    y = vec_ref[V_Y] + vec_ref[V_GA] * _sub_allreduce(part)
    m1 = vec_ref[V_X, :, pl.ds(0, 128)]
    st = vec_ref[V_SB]
    g = vec_ref[V_CB]
    yg = y * g
    a0, a1, a2 = _lane_mean(y), _lane_mean(y * y), _lane_mean(yg)
    a3, a4, a5 = _lane_mean(yg * yg), _lane_mean(yg * g), _lane_mean(yg * st)
    g1, g2, gs = (vec_ref[V_MISC, :, pl.ds(c, 128)] for c in (256, 384, 512))
    r1 = lax.rsqrt(jnp.maximum(a1 - a0 * a0 + EPS, EPS))
    m2 = a2 - a0 * g1
    v2 = a3 - a0 * (2.0 * a4 - a0 * g2) - m2 * m2
    cv = a5 - a0 * gs
    r2 = lax.rsqrt(jnp.maximum(r1 * (r1 * v2 + 2.0 * cv) + vec_ref[V_MISC, :, pl.ds(128, 128)], EPS))
    r12 = r1 * r2
    hs = [(_tile(yg, t) - (_tile(g, t) * a0 + m2)) * r12 + _tile(st, t) * r2 for t in range(NT)]

    def tanh_unit(t, r0, n):
        a = w1c[pl.ds(r0, n), :].reshape(n // 8, 8, 128)
        b = b1c[pl.ds(r0, n), :].reshape(n // 8, 8, 128)
        v = hs[t][None] * a + b
        return jnp.tanh(v * (v * v + GELU_KAPPA)).reshape(n, 128)

    def reduce_unit(r0, n, th):
        return jnp.dot(ab_ref[:, pl.ds(r0, n)], th, preferred_element_type=F32, precision=lax.Precision.DEFAULT)

    units = [(t, r0, min(128, FF - NV - r0)) for r0 in range(0, FF - NV, 128) for t in range(NT)]
    acc = [vec_ref[V_MISC, :, pl.ds(0, 128)]] * NT
    for k, (t, r0, n) in enumerate(units[:MLP_SPLIT]):
        th = tanh_unit(t, r0, n)
        if k < MLP_SPLIT - KS:
            acc[t] = acc[t] + reduce_unit(r0, n, th)
        else:
            qb_ref[pl.ds((k - (MLP_SPLIT - KS)) * 128, n), :] = th
    wait(gb_v, gsem)
    for k, (t, r0, n) in enumerate(units[MLP_SPLIT - KS:MLP_SPLIT]):
        acc[t] = acc[t] + reduce_unit(r0, n, qb_ref[pl.ds(k * 128, n), :])
    gb = []
    for t, r0, n in units[MLP_SPLIT:]:
        acc[t] = acc[t] + reduce_unit(r0, n, tanh_unit(t, r0, n))
        w = gb_v[:, :, pl.ds(len(gb) * 128, 128)].reshape(D, 128)
        gb.append(jnp.dot(sc_ref[...], w, preferred_element_type=F32))
    row = lax.broadcasted_iota(jnp.int32, (8, 128), 0)
    accv = [None] * NT
    for r in range(FF - NV, FF, 8):
        a, b, w = w1c[pl.ds(r, 8), :], b1c[pl.ds(r, 8), :], w2c[pl.ds(r - (FF - 128), 8), :]
        for t in range(NT):
            v = hs[t] * a + b
            g = (v * jnp.tanh(v * (v * v + GELU_KAPPA))) * w
            accv[t] = g if accv[t] is None else accv[t] + g
    outs = []
    for t in range(NT):
        yt = acc[t] * jnp.where(row < 2, hs[t], 1.0) + accv[t]
        outs.append(_tile(y, t) + m1 + gb[t] * _sub_allreduce(yt))
    o_ref[0] = jnp.concatenate(outs, axis=1)[0:1, :].astype(o_ref.dtype)


@jax.jit
def pallas_adaLN_cond__sliding_block_cached__mixer_token_mlp__decode_kernel(
    A_x: jax.Array,
    A_k_cache: jax.Array,
    A_v_cache: jax.Array,
    A_wq: jax.Array,
    A_wo: jax.Array,
    B_x: jax.Array,
    B_w1: jax.Array,
    B_b1: jax.Array,
    B_w2: jax.Array,
    B_b2: jax.Array,
    c: jax.Array,
    w_mod: jax.Array,
):
    del B_x
    kt = jnp.swapaxes(A_k_cache, 2, 3).reshape(H * DH, SK)
    vt = jnp.swapaxes(A_v_cache, 2, 3).reshape(H * DH, SK)

    def tiles(w):
        return w.reshape(w.shape[0] // 8, 8, w.shape[1] // 128, 128).transpose(0, 2, 1, 3).reshape(GF, RF, 128)

    args = (A_x.reshape(1, D), kt, vt, tiles(A_wq), tiles(A_wo), B_w1,
            B_b1.reshape(NC, 128), B_w2.reshape(1, FF), B_b2, c, w_mod.reshape(GM, RM, 6 * D))
    scratch = [
        pltpu.VMEM((NB, DH, CB), BF16),
        pltpu.VMEM((NB, DH, CB), BF16),
        pltpu.VMEM((GF, RF, 128), BF16),
        pltpu.VMEM((GF, RF, 128), BF16),
        pltpu.VMEM((GM, RM, WM_G * D), BF16),
        pltpu.VMEM((GM, RM, D), BF16),
        pltpu.VMEM((1, D), BF16),
        pltpu.VMEM((1, D), BF16),
        pltpu.VMEM((1, FF), BF16),
        pltpu.VMEM((NC, 128), BF16),
        pltpu.VMEM((1, FF), BF16),
        pltpu.VMEM((1,), BF16),
        pltpu.VMEM((KS * 128, 128), F32),
        pltpu.VMEM((NB, 8, CB), F32),
        pltpu.VMEM((NB, 8, CB), F32),
        pltpu.VMEM((8, D), F32),
        pltpu.VMEM((9, 8, D), F32),
        pltpu.VMEM((8, D), BF16),
        pltpu.VMEM((8, D), BF16),
        pltpu.VMEM((FF, 128), F32),
        pltpu.VMEM((FF, 128), F32),
        pltpu.VMEM((128, 128), F32),
        pltpu.VMEM((8, FF), F32),
        pltpu.SemaphoreType.DMA((NS,)),
        pltpu.SemaphoreType.DMA((NB,)),
        pltpu.SemaphoreType.DMA((6,)),
        pltpu.SemaphoreType.DMA(()),
    ]
    return pl.pallas_call(
        _kernel,
        in_specs=[pl.BlockSpec(memory_space=pl.ANY)] * len(args),
        out_specs=pl.BlockSpec(memory_space=pltpu.VMEM),
        out_shape=jax.ShapeDtypeStruct((1, 1, D), BF16),
        scratch_shapes=scratch,
        compiler_params=pltpu.CompilerParams(
            vmem_limit_bytes=120 * 1024 * 1024,
            disable_bounds_checks=True,
            disable_semaphore_checks=True,
        ),
    )(*args)
```

```python
import functools

import jax
import jax.numpy as jnp
from jax import lax
import jax.experimental.pallas as pl
import jax.experimental.pallas.tpu as pltpu

F32 = jnp.float32
BF16 = jnp.bfloat16

D = 640
H = 32
DH = 192
SK = 32768
W = 4096
FF = 1536
EPS = 1e-5
NT = D // 128
NC = FF // 128
NG = DH // 8

CB = 128
NB = W // CB
HR = 16

NS = 16
GM = 10
RM = D // GM
GH = 2
WM_G = 5
WM_STEPS = WM_G * (RM // 8)
GF = 15
RF = D * H * DH // (128 * GF)
F_STEPS = RF // 8
SEG = 4
SEGF = 14

DR = 64
ND = 2
DG = ND * DR // 8
SPV = 64

MLP_SPLIT = 55
KS = 5
NV = 96

GELU_K0 = 0.7978845608028654
GELU_K1 = GELU_K0 * 0.044715
GELU_S = GELU_K1 ** (1.0 / 3.0)
GELU_KAPPA = GELU_K0 / GELU_S

V_X, V_XN, V_SA, V_CA, V_GA, V_SB, V_CB, V_Y, V_MISC = range(9)


def _lane_mean(v):
    return jnp.sum(v, axis=-1, keepdims=True) * (1.0 / D)


def _col_bcast(row):
    return jnp.broadcast_to(row, (128, 128)).T


def _chain_sum(xs, n):
    chains = [functools.reduce(lambda a, b: a + b, xs[i::n]) for i in range(n)]
    while len(chains) > 1:
        chains = [chains[i] + chains[i + 1] for i in range(0, len(chains), 2)]
    return chains[0]


def _sub_allreduce(v):
    v = v + pltpu.roll(v, 4, 0)
    v = v + pltpu.roll(v, 2, 0)
    return v + pltpu.roll(v, 1, 0)


def _tile(v, t):
    return v[:, t * 128:(t + 1) * 128]


def _mult(i, n):
    return i if isinstance(i, int) else pl.multiple_of(i, n)


def _rem(i, n):
    if isinstance(i, int):
        return i % n
    return i & (n - 1) if n & (n - 1) == 0 else lax.rem(i, n)


def _div(i, n):
    if isinstance(i, int):
        return i // n
    return i >> (n.bit_length() - 1) if n & (n - 1) == 0 else lax.div(i, n)


def _kernel(x_hbm, k_hbm, v_hbm, wq_hbm, wo_hbm, w1_hbm, b1_hbm, w2_hbm, b2_hbm, c_hbm, wm_hbm,
            o_ref,
            kbuf, vbuf, wq_v, wo_v, wm_v, gb_v, x_v, c_v, w1_v, b1_v, w2_v, b2_v,
            qb_ref, s_ref, p_ref, attn_ref, vec_ref, sc_ref, h8_ref, w1c, b1c, w2c, ab_ref,
            sems, kvs, ssems, gsem):

    def dma(src, dst, sem, prio):
        pltpu.make_async_copy(src, dst, sem).start(priority=prio)

    def wait(dst, sem):
        pltpu.make_async_copy(dst, dst, sem).wait()

    def steps(hbm, vmem, groups, where, sem):
        def issue(i, which=(0, 1)):
            idx = where(i)
            for g, prio in ((pl.ds(0, GH), 0), (pl.ds(GH, groups - GH), 1)):
                if prio in which:
                    dma(hbm.at[(g,) + idx], vmem.at[(g,) + idx], sem(i), prio)

        def wait_(i):
            wait(vmem.at[(pl.ds(0, groups),) + where(i)], sem(i))

        return issue, wait_

    wm_issue, wm_wait = steps(
        wm_hbm, wm_v, GM,
        lambda i: (pl.ds(_mult(_div(i, WM_G) * 8, 8), 8), pl.ds(_mult(_rem(i, WM_G) * D, 128), D)),
        lambda i: sems.at[_rem(i, NS)])

    def flat_steps(hbm, vmem, groups):
        return steps(hbm, vmem, groups, lambda i: (pl.ds(_mult(i * 8, 8), 8), slice(None)),
                     lambda i: kvs.at[_rem(i, NB)])

    wq_issue, wq_wait = flat_steps(wq_hbm, wq_v, GF)
    wo_issue, wo_wait = flat_steps(wo_hbm, wo_v, GF)
    wos_issue, wos_wait = flat_steps(wo_hbm, wo_v, GF - 1)
    TG = RF // 8

    def tile_at(t0, lo, hi, t):
        if (t0 + lo) // TG == (t0 + hi) // TG:
            g = (t0 + lo) // TG
            return g, _mult((t0 - g * TG) * 8 + t * 8, 8)
        return _div(t0 + t, TG), _mult(_rem(t0 + t, TG) * 8, 8)

    def kv_issue(src, buf, h, j):
        c = pl.ds(_mult(SK - W + j * CB, 128), CB)
        dma(src.at[pl.ds(_mult(h * DH, 8), HR), c], buf.at[j, pl.ds(0, HR), :], kvs.at[j], 0)
        dma(src.at[pl.ds(_mult(h * DH + HR, 8), DH - HR), c], buf.at[j, pl.ds(HR, DH - HR), :], kvs.at[j], 1)

    def wq0_issue(j):
        for u in range(NB // NS):
            wq_issue(j * (NB // NS) + u)

    def end_issue(j):
        @pl.when(j < ND)
        def _():
            r = pl.ds(pl.multiple_of(RF - (ND - j) * DR * NT, 8), DR * NT)
            dma(wo_hbm.at[GF - 1, r, :], wo_v.at[GF - 1, r, :], sems.at[j], 1)

        @pl.when(j == ND)
        def _():
            for r in range(0, RM, 8):
                dma(wm_hbm.at[:, pl.ds(r, 8), pl.ds(WM_G * D, D)], gb_v.at[:, pl.ds(r, 8), :], gsem, 1)

    def pump(lo, hi, wait_fn, issue_fn, off):
        def body(i, carry):
            wait_fn(i)
            issue_fn(i + off)
            return carry
        lax.fori_loop(lo, hi, body, 0)

    def phase(n, wait_fn, issue_fn, next_issue, tasks, win, seg):
        for k, task in enumerate(tasks):
            pump(k * seg, (k + 1) * seg, wait_fn, issue_fn, win)
            task()
        pump(len(tasks) * seg, n - win, wait_fn, issue_fn, win)
        pump(n - win, n, wait_fn, next_issue, win - n)

    for i in range(NS):
        wm_issue(i, (1,))
    small = [pltpu.make_async_copy(s, d, ssems.at[n]) for n, (s, d) in enumerate(
        [(c_hbm, c_v), (x_hbm, x_v), (w1_hbm, w1_v), (b1_hbm, b1_v), (w2_hbm, w2_v), (b2_hbm, b2_v)])]
    for cp in small:
        cp.start()

    def spaced(i, carry):
        wm_issue(i, (0,))
        w1c[pl.ds(0, SPV * 8), :] = jnp.full((SPV * 8, 128), i, jnp.int32).astype(F32)
        return carry

    lax.fori_loop(0, NS, spaced, 0)

    def first_task():
        for cp in small:
            cp.wait()
        c = c_v[...].astype(F32)
        sc_ref[...] = jnp.broadcast_to(c * jax.nn.sigmoid(c), (8, D)).astype(BF16)
        x8 = jnp.broadcast_to(x_v[...].astype(F32), (8, D))
        xc = x8 - _lane_mean(x8)
        vec_ref[V_X] = x8
        vec_ref[V_XN] = xc * lax.rsqrt(_lane_mean(xc * xc) + EPS)
        attn_ref[...] = jnp.zeros(attn_ref.shape, F32)
        w2f = w2_v[...].astype(F32) * 0.5
        w1r = w1_v[...].astype(F32)
        b1r = b1_v[...].astype(F32)
        row = lax.broadcasted_iota(jnp.int32, (8, 128), 0)
        sum_ab = jnp.zeros((8, 128), F32)
        for b in range(NC):
            wa = _tile(w2f, b) * _tile(w1r, b)
            wb = _tile(w2f, b) * b1r[b:b + 1, :]
            ab = jnp.where(row < 2, jnp.broadcast_to(wa, (8, 128)), jnp.broadcast_to(wb, (8, 128)))
            ab = jnp.where(row < 4, ab, 0.0)
            hi = ab.astype(BF16).astype(F32)
            ab_ref[:, pl.ds(b * 128, 128)] = jnp.where(row % 2 == 0, hi, (ab - hi).astype(BF16).astype(F32))
            sum_ab = sum_ab + jnp.where(row % 2 == 0, ab, 0.0)
        sum_ab = jnp.broadcast_to(jnp.sum(sum_ab, axis=1, keepdims=True), (8, 128))
        b2 = jnp.broadcast_to(b2_v[...].astype(F32), (8, 128))
        vec_ref[V_MISC, :, pl.ds(0, 128)] = sum_ab + jnp.where(row == 2, b2, 0.0)

    def col_task(b0, nb):
        def task():
            w1f = w1_v[...].astype(F32) * GELU_S
            b1f = b1_v[...].astype(F32) * GELU_S
            for b in range(b0, b0 + nb):
                w1c[pl.ds(b * 128, 128), :] = _col_bcast(_tile(w1f, b))
                b1c[pl.ds(b * 128, 128), :] = _col_bcast(b1f[b:b + 1, :])
            if b0 == 0:
                w2c[...] = _col_bcast(_tile(w2_v[...].astype(F32) * (0.5 / GELU_S), NC - 1))
        return task

    def mod_task(n):
        def task():
            w = wm_v[:, :, pl.ds(n * D, D)].reshape(D, D)
            vec_ref[V_SA + n] = jnp.dot(sc_ref[...], w, preferred_element_type=F32)
        return task

    def h_task():
        h8_ref[...] = (vec_ref[V_XN] * (1.0 + vec_ref[V_CA]) + vec_ref[V_SA]).astype(BF16)
        sb = vec_ref[V_SB]
        st = sb - _lane_mean(sb)
        vec_ref[V_SB] = st
        g = 1.0 + vec_ref[V_CB]
        vec_ref[V_CB] = g
        vec_ref[V_MISC, :, pl.ds(256, 128)] = jnp.broadcast_to(_lane_mean(g), (8, 128))
        vec_ref[V_MISC, :, pl.ds(384, 128)] = jnp.broadcast_to(_lane_mean(g * g), (8, 128))
        vec_ref[V_MISC, :, pl.ds(512, 128)] = jnp.broadcast_to(_lane_mean(g * st), (8, 128))
        vec_ref[V_MISC, :, pl.ds(128, 128)] = jnp.broadcast_to(_lane_mean(st * st) + EPS, (8, 128))

    def q_cols(h):
        c0 = _div(h * DH, 128)
        for b in range(2):
            nct = H * DH // 128
            at = [tile_at(r * nct, 0, nct - 1, c0 + b) for r in range(D // 8)]
            w = jnp.concatenate([wq_v[g, pl.ds(r, 8), :] for g, r in at], axis=0)
            q = jnp.dot(h8_ref[...], w, preferred_element_type=F32)
            q = q.astype(BF16).astype(F32) * (DH ** -0.5)
            qb_ref[pl.ds(b * 128, 128), :] = _col_bcast(q[0:1])

    phase(WM_STEPS, wm_wait, wm_issue, wq0_issue, [first_task], NS, SEG)
    phase(F_STEPS, wq_wait, wq_issue, wo_issue,
          [mod_task(n) for n in range(WM_G)] + [h_task] + [col_task(b, 2) for b in range(0, NC, 2)], NB, SEGF)
    nfull = F_STEPS - DG * NT
    phase(nfull, wo_wait, wo_issue, lambda i: wos_issue(i + nfull), [lambda: q_cols(0)], NB, SEGF)
    pump(nfull, F_STEPS - NB, wos_wait, wos_issue, NB)
    pump(F_STEPS - NB, F_STEPS, wos_wait, lambda j: kv_issue(k_hbm, kbuf, 0, j), NB - F_STEPS)

    def scores(h, issue):
        r0 = _mult(_rem(h * DH, 128), 64)

        def kstep(j, carry):
            wait(kbuf.at[j], kvs.at[j])
            issue(j)
            parts = []
            for g in range(NG // 2):
                kg = kbuf[j, pl.ds(g * 16, 16), :].astype(F32)
                for rr in range(2):
                    parts.append(kg[rr * 8:rr * 8 + 8] * qb_ref[pl.ds(r0 + g * 16 + rr * 8, 8), :])
            s_ref[j] = _chain_sum(parts, 4)
            return carry

        lax.fori_loop(0, NB, kstep, 0)

        s = jnp.sum(s_ref[...], axis=1, keepdims=True)
        m = jnp.max(jnp.max(s, axis=0), axis=1, keepdims=True)
        p = jnp.exp(s - m[None])
        l = jnp.sum(jnp.sum(p, axis=0), axis=1, keepdims=True)
        p_ref[...] = jnp.broadcast_to(p, p_ref.shape)
        return 1.0 / l

    def values(issue):
        def vstep(j, acc):
            wait(vbuf.at[j], kvs.at[j])
            issue(j)
            pj = p_ref[j]
            out = []
            for g in range(NG // 2):
                vg = vbuf[j, pl.ds(g * 16, 16), :].astype(F32)
                for rr in range(2):
                    out.append(acc[2 * g + rr] + vg[rr * 8:rr * 8 + 8] * pj)
            return tuple(out)

        return lax.fori_loop(0, NB, vstep, tuple(jnp.zeros((8, 128), F32) for _ in range(NG)))

    def project(rt0, og, lo=0, hi=H * NG):
        terms = [[] for _ in range(NT)]
        for blk in range(len(og) * NT // 8):
            g, r = tile_at(blk * 8, lo * NT, hi * NT, rt0 * NT)
            r = _mult(r, 64)
            for k in range(4):
                w = wo_v[g, pl.ds(r + k * 16, 16), :].astype(F32)
                for e in range(2):
                    u = blk * 8 + 2 * k + e
                    terms[u % NT].append(w[e * 8:e * 8 + 8] * og[u // NT])
        return jnp.concatenate([_chain_sum(ts, 2) for ts in terms], axis=1)

    def head_body(h, carry):
        inv_l = scores(h, lambda j: kv_issue(v_hbm, vbuf, h, j))
        q_cols(h + 1)
        acc = values(lambda j: kv_issue(k_hbm, kbuf, h + 1, j))
        og = [jnp.sum(a, axis=1, keepdims=True) * inv_l for a in acc]
        attn_ref[...] += project(h * NG, og)
        return carry

    lax.fori_loop(0, H - 1, head_body, 0)

    inv_l = scores(H - 1, lambda j: kv_issue(v_hbm, vbuf, H - 1, j))
    xp = vec_ref[V_X] + vec_ref[V_GA] * _sub_allreduce(attn_ref[...])
    mp = _lane_mean(xp)
    vec_ref[V_Y] = xp - mp
    vec_ref[V_X, :, pl.ds(0, 128)] = jnp.broadcast_to(mp, (8, 128))
    acc = values(end_issue)
    og = [jnp.sum(a, axis=1, keepdims=True) * inv_l for a in acc]
    for g in range(DG):
        s_ref[g] = jnp.broadcast_to(og[NG - DG + g], (8, 128))
    part = project((H - 1) * NG, og[:NG - DG])

    def dstep(i, part):
        r = pl.ds(pl.multiple_of(RF - (ND - i) * DR * NT, 8), DR * NT)
        wait(wo_v.at[GF - 1, r, :], sems.at[i])
        g0 = i * (DR // 8)
        og = [s_ref[g0 + g] for g in range(DR // 8)]
        return part + project(H * NG - DG + g0, og, H * NG - DG, H * NG - DR // 8)

    part = lax.fori_loop(0, ND, dstep, part)

    y = vec_ref[V_Y] + vec_ref[V_GA] * _sub_allreduce(part)
    m1 = vec_ref[V_X, :, pl.ds(0, 128)]
    st = vec_ref[V_SB]
    g = vec_ref[V_CB]
    yg = y * g
    a0, a1, a2 = _lane_mean(y), _lane_mean(y * y), _lane_mean(yg)
    a3, a4, a5 = _lane_mean(yg * yg), _lane_mean(yg * g), _lane_mean(yg * st)
    g1, g2, gs = (vec_ref[V_MISC, :, pl.ds(c, 128)] for c in (256, 384, 512))
    r1 = lax.rsqrt(jnp.maximum(a1 - a0 * a0 + EPS, EPS))
    m2 = a2 - a0 * g1
    v2 = a3 - a0 * (2.0 * a4 - a0 * g2) - m2 * m2
    cv = a5 - a0 * gs
    r2 = lax.rsqrt(jnp.maximum(r1 * (r1 * v2 + 2.0 * cv) + vec_ref[V_MISC, :, pl.ds(128, 128)], EPS))
    r12 = r1 * r2
    hs = [(_tile(yg, t) - (_tile(g, t) * a0 + m2)) * r12 + _tile(st, t) * r2 for t in range(NT)]

    def tanh_unit(t, r0, n):
        a = w1c[pl.ds(r0, n), :].reshape(n // 8, 8, 128)
        b = b1c[pl.ds(r0, n), :].reshape(n // 8, 8, 128)
        v = hs[t][None] * a + b
        return jnp.tanh(v * (v * v + GELU_KAPPA)).reshape(n, 128)

    def reduce_unit(r0, n, th):
        return jnp.dot(ab_ref[:, pl.ds(r0, n)], th, preferred_element_type=F32, precision=lax.Precision.DEFAULT)

    units = [(t, r0, min(128, FF - NV - r0)) for r0 in range(0, FF - NV, 128) for t in range(NT)]
    acc = [vec_ref[V_MISC, :, pl.ds(0, 128)]] * NT
    for k, (t, r0, n) in enumerate(units[:MLP_SPLIT]):
        th = tanh_unit(t, r0, n)
        if k < MLP_SPLIT - KS:
            acc[t] = acc[t] + reduce_unit(r0, n, th)
        else:
            qb_ref[pl.ds((k - (MLP_SPLIT - KS)) * 128, n), :] = th
    wait(gb_v, gsem)
    for k, (t, r0, n) in enumerate(units[MLP_SPLIT - KS:MLP_SPLIT]):
        acc[t] = acc[t] + reduce_unit(r0, n, qb_ref[pl.ds(k * 128, n), :])
    gb = []
    for t, r0, n in units[MLP_SPLIT:]:
        acc[t] = acc[t] + reduce_unit(r0, n, tanh_unit(t, r0, n))
        w = gb_v[:, :, pl.ds(len(gb) * 128, 128)].reshape(D, 128)
        gb.append(jnp.dot(sc_ref[...], w, preferred_element_type=F32))
    row = lax.broadcasted_iota(jnp.int32, (8, 128), 0)
    accv = [None] * NT
    for r in range(FF - NV, FF, 8):
        a, b, w = w1c[pl.ds(r, 8), :], b1c[pl.ds(r, 8), :], w2c[pl.ds(r - (FF - 128), 8), :]
        for t in range(NT):
            v = hs[t] * a + b
            g = (v * jnp.tanh(v * (v * v + GELU_KAPPA))) * w
            accv[t] = g if accv[t] is None else accv[t] + g
    outs = []
    for t in range(NT):
        yt = acc[t] * jnp.where(row < 2, hs[t], 1.0) + accv[t]
        outs.append(_tile(y, t) + m1 + gb[t] * _sub_allreduce(yt))
    o_ref[0] = jnp.concatenate(outs, axis=1)[0:1, :].astype(o_ref.dtype)


@jax.jit
def pallas_adaLN_cond__sliding_block_cached__mixer_token_mlp__decode_kernel(
    A_x: jax.Array,
    A_k_cache: jax.Array,
    A_v_cache: jax.Array,
    A_wq: jax.Array,
    A_wo: jax.Array,
    B_x: jax.Array,
    B_w1: jax.Array,
    B_b1: jax.Array,
    B_w2: jax.Array,
    B_b2: jax.Array,
    c: jax.Array,
    w_mod: jax.Array,
):
    del B_x
    kt = jnp.swapaxes(A_k_cache, 2, 3).reshape(H * DH, SK)
    vt = jnp.swapaxes(A_v_cache, 2, 3).reshape(H * DH, SK)

    def tiles(w):
        return w.reshape(w.shape[0] // 8, 8, w.shape[1] // 128, 128).transpose(0, 2, 1, 3).reshape(GF, RF, 128)

    args = (A_x.reshape(1, D), kt, vt, tiles(A_wq), tiles(A_wo), B_w1,
            B_b1.reshape(NC, 128), B_w2.reshape(1, FF), B_b2, c, w_mod.reshape(GM, RM, 6 * D))
    scratch = [
        pltpu.VMEM((NB, DH, CB), BF16),
        pltpu.VMEM((NB, DH, CB), BF16),
        pltpu.VMEM((GF, RF, 128), BF16),
        pltpu.VMEM((GF, RF, 128), BF16),
        pltpu.VMEM((GM, RM, WM_G * D), BF16),
        pltpu.VMEM((GM, RM, D), BF16),
        pltpu.VMEM((1, D), BF16),
        pltpu.VMEM((1, D), BF16),
        pltpu.VMEM((1, FF), BF16),
        pltpu.VMEM((NC, 128), BF16),
        pltpu.VMEM((1, FF), BF16),
        pltpu.VMEM((1,), BF16),
        pltpu.VMEM((KS * 128, 128), F32),
        pltpu.VMEM((NB, 8, CB), F32),
        pltpu.VMEM((NB, 8, CB), F32),
        pltpu.VMEM((8, D), F32),
        pltpu.VMEM((9, 8, D), F32),
        pltpu.VMEM((8, D), BF16),
        pltpu.VMEM((8, D), BF16),
        pltpu.VMEM((FF, 128), F32),
        pltpu.VMEM((FF, 128), F32),
        pltpu.VMEM((128, 128), F32),
        pltpu.VMEM((8, FF), F32),
        pltpu.SemaphoreType.DMA((NS,)),
        pltpu.SemaphoreType.DMA((NB,)),
        pltpu.SemaphoreType.DMA((6,)),
        pltpu.SemaphoreType.DMA(()),
    ]
    return pl.pallas_call(
        _kernel,
        in_specs=[pl.BlockSpec(memory_space=pl.ANY)] * len(args),
        out_specs=pl.BlockSpec(memory_space=pltpu.VMEM),
        out_shape=jax.ShapeDtypeStruct((1, 1, D), BF16),
        scratch_shapes=scratch,
        compiler_params=pltpu.CompilerParams(
            vmem_limit_bytes=120 * 1024 * 1024,
            disable_bounds_checks=True,
            disable_semaphore_checks=True,
        ),
    )(*args)
```

```python
import functools

import jax
import jax.numpy as jnp
from jax import lax
import jax.experimental.pallas as pl
import jax.experimental.pallas.tpu as pltpu

F32 = jnp.float32
BF16 = jnp.bfloat16

D = 640
H = 32
DH = 192
SK = 32768
W = 4096
FF = 1536
EPS = 1e-5
NT = D // 128
NC = FF // 128
NG = DH // 8

CB = 128
NB = W // CB
HR = 16

NS = 16
GM = 10
RM = D // GM
GH = 2
WM_G = 5
WM_STEPS = WM_G * (RM // 8)
GF = 15
RF = D * H * DH // (128 * GF)
F_STEPS = RF // 8
SEG = 4
SEGF = 14

DR = 64
ND = 2
DG = ND * DR // 8
SPV = 64

MLP_SPLIT = 55
KS = 5
NV = 96

GELU_K0 = 0.7978845608028654
GELU_K1 = GELU_K0 * 0.044715
GELU_S = GELU_K1 ** (1.0 / 3.0)
GELU_KAPPA = GELU_K0 / GELU_S

V_X, V_XN, V_SA, V_CA, V_GA, V_SB, V_CB, V_Y, V_MISC = range(9)


def _lane_mean(v):
    return jnp.sum(v, axis=-1, keepdims=True) * (1.0 / D)


def _col_bcast(row):
    return jnp.broadcast_to(row, (128, 128)).T


def _chain_sum(xs, n):
    chains = [functools.reduce(lambda a, b: a + b, xs[i::n]) for i in range(n)]
    while len(chains) > 1:
        chains = [chains[i] + chains[i + 1] for i in range(0, len(chains), 2)]
    return chains[0]


def _sub_allreduce(v):
    v = v + pltpu.roll(v, 4, 0)
    v = v + pltpu.roll(v, 2, 0)
    return v + pltpu.roll(v, 1, 0)


def _tile(v, t):
    return v[:, t * 128:(t + 1) * 128]


def _mult(i, n):
    return i if isinstance(i, int) else pl.multiple_of(i, n)


def _rem(i, n):
    if isinstance(i, int):
        return i % n
    return i & (n - 1) if n & (n - 1) == 0 else lax.rem(i, n)


def _div(i, n):
    if isinstance(i, int):
        return i // n
    return i >> (n.bit_length() - 1) if n & (n - 1) == 0 else lax.div(i, n)


def _kernel(x_hbm, k_hbm, v_hbm, wq_hbm, wo_hbm, w1_hbm, b1_hbm, w2_hbm, b2_hbm, c_hbm, wm_hbm,
            o_ref,
            kbuf, vbuf, wq_v, wo_v, wm_v, gb_v, x_v, c_v, w1_v, b1_v, w2_v, b2_v,
            qb_ref, s_ref, p_ref, attn_ref, vec_ref, sc_ref, h8_ref, w1c, b1c, w2c, ab_ref,
            sems, kvs, ssems, gsem):

    def dma(src, dst, sem, prio):
        pltpu.make_async_copy(src, dst, sem).start(priority=prio)

    def wait(dst, sem):
        pltpu.make_async_copy(dst, dst, sem).wait()

    def steps(hbm, vmem, groups, where, sem):
        def issue(i, which=(0, 1)):
            idx = where(i)
            for g, prio in ((pl.ds(0, GH), 0), (pl.ds(GH, groups - GH), 1)):
                if prio in which:
                    dma(hbm.at[(g,) + idx], vmem.at[(g,) + idx], sem(i), prio)

        def wait_(i):
            wait(vmem.at[(pl.ds(0, groups),) + where(i)], sem(i))

        return issue, wait_

    wm_issue, wm_wait = steps(
        wm_hbm, wm_v, GM,
        lambda i: (pl.ds(_mult(_div(i, WM_G) * 8, 8), 8), pl.ds(_mult(_rem(i, WM_G) * D, 128), D)),
        lambda i: sems.at[_rem(i, NS)])

    def flat_steps(hbm, vmem, groups):
        return steps(hbm, vmem, groups, lambda i: (pl.ds(_mult(i * 8, 8), 8), slice(None)),
                     lambda i: kvs.at[_rem(i, NB)])

    wq_issue, wq_wait = flat_steps(wq_hbm, wq_v, GF)
    wo_issue, wo_wait = flat_steps(wo_hbm, wo_v, GF)
    wos_issue, wos_wait = flat_steps(wo_hbm, wo_v, GF - 1)
    TG = RF // 8

    def tile_at(t0, lo, hi, t):
        if (t0 + lo) // TG == (t0 + hi) // TG:
            g = (t0 + lo) // TG
            return g, _mult((t0 - g * TG) * 8 + t * 8, 8)
        return _div(t0 + t, TG), _mult(_rem(t0 + t, TG) * 8, 8)

    def kv_issue(src, buf, h, j):
        c = pl.ds(_mult(SK - W + j * CB, 128), CB)
        dma(src.at[pl.ds(_mult(h * DH, 8), HR), c], buf.at[j, pl.ds(0, HR), :], kvs.at[j], 0)
        dma(src.at[pl.ds(_mult(h * DH + HR, 8), DH - HR), c], buf.at[j, pl.ds(HR, DH - HR), :], kvs.at[j], 1)

    def wq0_issue(j):
        for u in range(NB // NS):
            wq_issue(j * (NB // NS) + u)

    def end_issue(j):
        @pl.when(j < ND)
        def _():
            r = pl.ds(pl.multiple_of(RF - (ND - j) * DR * NT, 8), DR * NT)
            dma(wo_hbm.at[GF - 1, r, :], wo_v.at[GF - 1, r, :], sems.at[j], 1)

        @pl.when(j == ND)
        def _():
            for r in range(0, RM, 8):
                dma(wm_hbm.at[:, pl.ds(r, 8), pl.ds(WM_G * D, D)], gb_v.at[:, pl.ds(r, 8), :], gsem, 1)

    def pump(lo, hi, wait_fn, issue_fn, off):
        def body(i, carry):
            wait_fn(i)
            issue_fn(i + off)
            return carry
        lax.fori_loop(lo, hi, body, 0)

    def phase(n, wait_fn, issue_fn, next_issue, tasks, win, seg):
        for k, task in enumerate(tasks):
            pump(k * seg, (k + 1) * seg, wait_fn, issue_fn, win)
            task()
        pump(len(tasks) * seg, n - win, wait_fn, issue_fn, win)
        pump(n - win, n, wait_fn, next_issue, win - n)

    for i in range(NS):
        wm_issue(i, (1,))
    small = [pltpu.make_async_copy(s, d, ssems.at[n]) for n, (s, d) in enumerate(
        [(c_hbm, c_v), (x_hbm, x_v), (w1_hbm, w1_v), (b1_hbm, b1_v), (w2_hbm, w2_v), (b2_hbm, b2_v)])]
    for cp in small:
        cp.start()

    def spaced(i, carry):
        wm_issue(i, (0,))
        w1c[pl.ds(0, SPV * 8), :] = jnp.full((SPV * 8, 128), i, jnp.int32).astype(F32)
        return carry

    lax.fori_loop(0, NS, spaced, 0)

    def first_task():
        for cp in small:
            cp.wait()
        c = c_v[...].astype(F32)
        sc_ref[...] = jnp.broadcast_to(c * jax.nn.sigmoid(c), (8, D)).astype(BF16)
        x8 = jnp.broadcast_to(x_v[...].astype(F32), (8, D))
        xc = x8 - _lane_mean(x8)
        vec_ref[V_X] = x8
        vec_ref[V_XN] = xc * lax.rsqrt(_lane_mean(xc * xc) + EPS)
        attn_ref[...] = jnp.zeros(attn_ref.shape, F32)
        w2f = w2_v[...].astype(F32) * 0.5
        w1r = w1_v[...].astype(F32)
        b1r = b1_v[...].astype(F32)
        row = lax.broadcasted_iota(jnp.int32, (8, 128), 0)
        sum_ab = jnp.zeros((8, 128), F32)
        for b in range(NC):
            wa = _tile(w2f, b) * _tile(w1r, b)
            wb = _tile(w2f, b) * b1r[b:b + 1, :]
            ab = jnp.where(row < 2, jnp.broadcast_to(wa, (8, 128)), jnp.broadcast_to(wb, (8, 128)))
            ab = jnp.where(row < 4, ab, 0.0)
            hi = ab.astype(BF16).astype(F32)
            ab_ref[:, pl.ds(b * 128, 128)] = jnp.where(row % 2 == 0, hi, (ab - hi).astype(BF16).astype(F32))
            sum_ab = sum_ab + jnp.where(row % 2 == 0, ab, 0.0)
        sum_ab = jnp.broadcast_to(jnp.sum(sum_ab, axis=1, keepdims=True), (8, 128))
        b2 = jnp.broadcast_to(b2_v[...].astype(F32), (8, 128))
        vec_ref[V_MISC, :, pl.ds(0, 128)] = sum_ab + jnp.where(row == 2, b2, 0.0)

    def col_task(b0, nb):
        def task():
            w1f = w1_v[...].astype(F32) * GELU_S
            b1f = b1_v[...].astype(F32) * GELU_S
            for b in range(b0, b0 + nb):
                w1c[pl.ds(b * 128, 128), :] = _col_bcast(_tile(w1f, b))
                b1c[pl.ds(b * 128, 128), :] = _col_bcast(b1f[b:b + 1, :])
            if b0 == 0:
                w2c[...] = _col_bcast(_tile(w2_v[...].astype(F32) * (0.5 / GELU_S), NC - 1))
        return task

    def mod_task(n):
        def task():
            w = wm_v[:, :, pl.ds(n * D, D)].reshape(D, D)
            vec_ref[V_SA + n] = jnp.dot(sc_ref[...], w, preferred_element_type=F32)
        return task

    def h_task():
        h8_ref[...] = (vec_ref[V_XN] * (1.0 + vec_ref[V_CA]) + vec_ref[V_SA]).astype(BF16)
        sb = vec_ref[V_SB]
        st = sb - _lane_mean(sb)
        vec_ref[V_SB] = st
        g = 1.0 + vec_ref[V_CB]
        vec_ref[V_CB] = g
        vec_ref[V_MISC, :, pl.ds(256, 128)] = jnp.broadcast_to(_lane_mean(g), (8, 128))
        vec_ref[V_MISC, :, pl.ds(384, 128)] = jnp.broadcast_to(_lane_mean(g * g), (8, 128))
        vec_ref[V_MISC, :, pl.ds(512, 128)] = jnp.broadcast_to(_lane_mean(g * st), (8, 128))
        vec_ref[V_MISC, :, pl.ds(128, 128)] = jnp.broadcast_to(_lane_mean(st * st) + EPS, (8, 128))

    def q_cols(h):
        c0 = _div(h * DH, 128)
        for b in range(2):
            nct = H * DH // 128
            at = [tile_at(r * nct, 0, nct - 1, c0 + b) for r in range(D // 8)]
            w = jnp.concatenate([wq_v[g, pl.ds(r, 8), :] for g, r in at], axis=0)
            q = jnp.dot(h8_ref[...], w, preferred_element_type=F32)
            q = q.astype(BF16).astype(F32) * (DH ** -0.5)
            qb_ref[pl.ds(b * 128, 128), :] = _col_bcast(q[0:1])

    phase(WM_STEPS, wm_wait, wm_issue, wq0_issue, [first_task], NS, SEG)
    phase(F_STEPS, wq_wait, wq_issue, wo_issue,
          [mod_task(n) for n in range(WM_G)] + [h_task] + [col_task(b, 2) for b in range(0, NC, 2)], NB, SEGF)
    nfull = F_STEPS - DG * NT
    phase(nfull, wo_wait, wo_issue, lambda i: wos_issue(i + nfull), [lambda: q_cols(0)], NB, SEGF)
    pump(nfull, F_STEPS - NB, wos_wait, wos_issue, NB)
    pump(F_STEPS - NB, F_STEPS, wos_wait, lambda j: kv_issue(k_hbm, kbuf, 0, j), NB - F_STEPS)

    def scores(h, issue):
        r0 = _mult(_rem(h * DH, 128), 64)

        def kstep(j, carry):
            wait(kbuf.at[j], kvs.at[j])
            issue(j)
            parts = []
            for g in range(NG // 2):
                kg = kbuf[j, pl.ds(g * 16, 16), :].astype(F32)
                for rr in range(2):
                    parts.append(kg[rr * 8:rr * 8 + 8] * qb_ref[pl.ds(r0 + g * 16 + rr * 8, 8), :])
            s_ref[j] = _chain_sum(parts, 4)
            return carry

        lax.fori_loop(0, NB, kstep, 0)

        s = jnp.sum(s_ref[...], axis=1, keepdims=True)
        m = jnp.max(jnp.max(s, axis=0), axis=1, keepdims=True)
        p = jnp.exp(s - m[None])
        l = jnp.sum(jnp.sum(p, axis=0), axis=1, keepdims=True)
        p_ref[...] = jnp.broadcast_to(p, p_ref.shape)
        return 1.0 / l

    def values(issue):
        def vstep(j, acc):
            wait(vbuf.at[j], kvs.at[j])
            issue(j)
            pj = p_ref[j]
            out = []
            for g in range(NG // 2):
                vg = vbuf[j, pl.ds(g * 16, 16), :].astype(F32)
                for rr in range(2):
                    out.append(acc[2 * g + rr] + vg[rr * 8:rr * 8 + 8] * pj)
            return tuple(out)

        return lax.fori_loop(0, NB, vstep, tuple(jnp.zeros((8, 128), F32) for _ in range(NG)))

    def project(rt0, og, lo=0, hi=H * NG):
        terms = [[] for _ in range(NT)]
        for blk in range(len(og) * NT // 8):
            g, r = tile_at(blk * 8, lo * NT, hi * NT, rt0 * NT)
            r = _mult(r, 64)
            for k in range(4):
                w = wo_v[g, pl.ds(r + k * 16, 16), :].astype(F32)
                for e in range(2):
                    u = blk * 8 + 2 * k + e
                    terms[u % NT].append(w[e * 8:e * 8 + 8] * og[u // NT])
        return jnp.concatenate([_chain_sum(ts, 2) for ts in terms], axis=1)

    def head_body(h, carry):
        inv_l = scores(h, lambda j: kv_issue(v_hbm, vbuf, h, j))
        q_cols(h + 1)
        acc = values(lambda j: kv_issue(k_hbm, kbuf, h + 1, j))
        og = [jnp.sum(a, axis=1, keepdims=True) * inv_l for a in acc]
        attn_ref[...] += project(h * NG, og)
        return carry

    lax.fori_loop(0, H - 1, head_body, 0)

    inv_l = scores(H - 1, lambda j: kv_issue(v_hbm, vbuf, H - 1, j))
    xp = vec_ref[V_X] + vec_ref[V_GA] * _sub_allreduce(attn_ref[...])
    mp = _lane_mean(xp)
    vec_ref[V_Y] = xp - mp
    vec_ref[V_X, :, pl.ds(0, 128)] = jnp.broadcast_to(mp, (8, 128))
    acc = values(end_issue)
    og = [jnp.sum(a, axis=1, keepdims=True) * inv_l for a in acc]
    for g in range(DG):
        s_ref[g] = jnp.broadcast_to(og[NG - DG + g], (8, 128))
    part = project((H - 1) * NG, og[:NG - DG])

    def dstep(i, part):
        r = pl.ds(pl.multiple_of(RF - (ND - i) * DR * NT, 8), DR * NT)
        wait(wo_v.at[GF - 1, r, :], sems.at[i])
        g0 = i * (DR // 8)
        og = [s_ref[g0 + g] for g in range(DR // 8)]
        return part + project(H * NG - DG + g0, og, H * NG - DG, H * NG - DR // 8)

    part = lax.fori_loop(0, ND, dstep, part)

    y = vec_ref[V_Y] + vec_ref[V_GA] * _sub_allreduce(part)
    m1 = vec_ref[V_X, :, pl.ds(0, 128)]
    st = vec_ref[V_SB]
    g = vec_ref[V_CB]
    yg = y * g
    a0, a1, a2 = _lane_mean(y), _lane_mean(y * y), _lane_mean(yg)
    a3, a4, a5 = _lane_mean(yg * yg), _lane_mean(yg * g), _lane_mean(yg * st)
    g1, g2, gs = (vec_ref[V_MISC, :, pl.ds(c, 128)] for c in (256, 384, 512))
    r1 = lax.rsqrt(jnp.maximum(a1 - a0 * a0 + EPS, EPS))
    m2 = a2 - a0 * g1
    v2 = a3 - a0 * (2.0 * a4 - a0 * g2) - m2 * m2
    cv = a5 - a0 * gs
    r2 = lax.rsqrt(jnp.maximum(r1 * (r1 * v2 + 2.0 * cv) + vec_ref[V_MISC, :, pl.ds(128, 128)], EPS))
    r12 = r1 * r2
    hs = [(_tile(yg, t) - (_tile(g, t) * a0 + m2)) * r12 + _tile(st, t) * r2 for t in range(NT)]

    def tanh_unit(t, r0, n):
        a = w1c[pl.ds(r0, n), :].reshape(n // 8, 8, 128)
        b = b1c[pl.ds(r0, n), :].reshape(n // 8, 8, 128)
        v = hs[t][None] * a + b
        return jnp.tanh(v * (v * v + GELU_KAPPA)).reshape(n, 128)

    def reduce_unit(r0, n, th):
        return jnp.dot(ab_ref[:, pl.ds(r0, n)], th, preferred_element_type=F32, precision=lax.Precision.DEFAULT)

    units = [(t, r0, min(128, FF - NV - r0)) for r0 in range(0, FF - NV, 128) for t in range(NT)]
    acc = [vec_ref[V_MISC, :, pl.ds(0, 128)]] * NT
    for k, (t, r0, n) in enumerate(units[:MLP_SPLIT]):
        th = tanh_unit(t, r0, n)
        if k < MLP_SPLIT - KS:
            acc[t] = acc[t] + reduce_unit(r0, n, th)
        else:
            qb_ref[pl.ds((k - (MLP_SPLIT - KS)) * 128, n), :] = th
    wait(gb_v, gsem)
    for k, (t, r0, n) in enumerate(units[MLP_SPLIT - KS:MLP_SPLIT]):
        acc[t] = acc[t] + reduce_unit(r0, n, qb_ref[pl.ds(k * 128, n), :])
    gb = []
    for t, r0, n in units[MLP_SPLIT:]:
        acc[t] = acc[t] + reduce_unit(r0, n, tanh_unit(t, r0, n))
        w = gb_v[:, :, pl.ds(len(gb) * 128, 128)].reshape(D, 128)
        gb.append(jnp.dot(sc_ref[...], w, preferred_element_type=F32))
    row = lax.broadcasted_iota(jnp.int32, (8, 128), 0)
    accv = [None] * NT
    for r in range(FF - NV, FF, 8):
        a, b, w = w1c[pl.ds(r, 8), :], b1c[pl.ds(r, 8), :], w2c[pl.ds(r - (FF - 128), 8), :]
        for t in range(NT):
            v = hs[t] * a + b
            g = (v * jnp.tanh(v * (v * v + GELU_KAPPA))) * w
            accv[t] = g if accv[t] is None else accv[t] + g
    outs = []
    for t in range(NT):
        yt = acc[t] * jnp.where(row < 2, hs[t], 1.0) + accv[t]
        outs.append(_tile(y, t) + m1 + gb[t] * _sub_allreduce(yt))
    o_ref[0] = jnp.concatenate(outs, axis=1)[0:1, :].astype(o_ref.dtype)


def _compiler_params():
    base = dict(vmem_limit_bytes=120 * 1024 * 1024, disable_bounds_checks=True)
    try:
        return pltpu.CompilerParams(disable_semaphore_checks=True, **base)
    except TypeError:
        return pltpu.CompilerParams(**base)


@jax.jit
def pallas_adaLN_cond__sliding_block_cached__mixer_token_mlp__decode_kernel(
    A_x: jax.Array,
    A_k_cache: jax.Array,
    A_v_cache: jax.Array,
    A_wq: jax.Array,
    A_wo: jax.Array,
    B_x: jax.Array,
    B_w1: jax.Array,
    B_b1: jax.Array,
    B_w2: jax.Array,
    B_b2: jax.Array,
    c: jax.Array,
    w_mod: jax.Array,
):
    del B_x
    kt = jnp.swapaxes(A_k_cache, 2, 3).reshape(H * DH, SK)
    vt = jnp.swapaxes(A_v_cache, 2, 3).reshape(H * DH, SK)

    def tiles(w):
        return w.reshape(w.shape[0] // 8, 8, w.shape[1] // 128, 128).transpose(0, 2, 1, 3).reshape(GF, RF, 128)

    args = (A_x.reshape(1, D), kt, vt, tiles(A_wq), tiles(A_wo), B_w1,
            B_b1.reshape(NC, 128), B_w2.reshape(1, FF), B_b2, c, w_mod.reshape(GM, RM, 6 * D))
    scratch = [
        pltpu.VMEM((NB, DH, CB), BF16),
        pltpu.VMEM((NB, DH, CB), BF16),
        pltpu.VMEM((GF, RF, 128), BF16),
        pltpu.VMEM((GF, RF, 128), BF16),
        pltpu.VMEM((GM, RM, WM_G * D), BF16),
        pltpu.VMEM((GM, RM, D), BF16),
        pltpu.VMEM((1, D), BF16),
        pltpu.VMEM((1, D), BF16),
        pltpu.VMEM((1, FF), BF16),
        pltpu.VMEM((NC, 128), BF16),
        pltpu.VMEM((1, FF), BF16),
        pltpu.VMEM((1,), BF16),
        pltpu.VMEM((KS * 128, 128), F32),
        pltpu.VMEM((NB, 8, CB), F32),
        pltpu.VMEM((NB, 8, CB), F32),
        pltpu.VMEM((8, D), F32),
        pltpu.VMEM((9, 8, D), F32),
        pltpu.VMEM((8, D), BF16),
        pltpu.VMEM((8, D), BF16),
        pltpu.VMEM((FF, 128), F32),
        pltpu.VMEM((FF, 128), F32),
        pltpu.VMEM((128, 128), F32),
        pltpu.VMEM((8, FF), F32),
        pltpu.SemaphoreType.DMA((NS,)),
        pltpu.SemaphoreType.DMA((NB,)),
        pltpu.SemaphoreType.DMA((6,)),
        pltpu.SemaphoreType.DMA(()),
    ]
    return pl.pallas_call(
        _kernel,
        in_specs=[pl.BlockSpec(memory_space=pl.ANY)] * len(args),
        out_specs=pl.BlockSpec(memory_space=pltpu.VMEM),
        out_shape=jax.ShapeDtypeStruct((1, 1, D), BF16),
        scratch_shapes=scratch,
        compiler_params=_compiler_params(),
    )(*args)
```
